```python
import jax
import jax.numpy as jnp

def _softmax(x, axis=-1):
    return jax.nn.softmax(x, axis=axis)

def _gelu(x):
    return jax.nn.gelu(x, approximate=True)

def _silu(x):
    return jax.nn.silu(x)

def _sigmoid(x):
    return jax.nn.sigmoid(x)

def _layernorm(x, axis=-1, eps=1e-05):
    m = jnp.mean(x, axis=axis, keepdims=True)
    v = jnp.var(x, axis=axis, keepdims=True)
    return (x - m) / jnp.sqrt(v + eps)

def _scatter_add(tgt, idx, src, axis=0):
    return tgt.at[idx].add(src)

def _segment_sum(src, seg, n):
    return jax.ops.segment_sum(src, seg, n)

class _Rng:

    def __init__(self, key):
        self._k = key

    def _next(self):
        self._k, sub = jax.random.split(self._k)
        return sub

    def normal(self, shape):
        return jax.random.normal(self._next(), shape, dtype=jnp.bfloat16)

    def randint(self, lo, hi, shape):
        return jax.random.randint(self._next(), shape, lo, hi, dtype=jnp.int32)

    def uniform(self, shape, lo=0.0, hi=1.0):
        return jax.random.uniform(self._next(), shape, jnp.bfloat16, lo, hi)

    def permutation(self, n):
        return jax.random.permutation(self._next(), n)
kernel_name = 'gated_mix__softmax_full_mha__memory_aug_recurrent_mem_tr__prompt'

def setup_inputs():
    _rng = _Rng(jax.random.key(int.from_bytes(__import__("os").urandom(4), "little")))
    _w = lambda a: (lambda t: t.astype(jnp.bfloat16) if jnp.issubdtype(t.dtype, jnp.floating) else t)(jnp.asarray(a))

    def _A_setup():
        B, S, D = (1, 2048, 1024)
        return {'x': _w((lambda *s: _rng.normal(s) * 0.05)(B, S, D)), 'wqkv': _w((lambda *s: _rng.normal(s) * 0.05)(D, 3 * D)), 'wo': _w((lambda *s: _rng.normal(s) * 0.05)(D, D))}
    _A_in = _A_setup()

    def _B_setup():
        B, S, Dm = (1, 2048, 1024)
        H, Dh = (32, 128)
        M, seg = (8, 32)
        seg = min(seg, S)
        S = S // seg * seg
        return {'x': _w((lambda *s: _rng.normal(s) * 0.05)(B, S, Dm)), 'mem0': _w((lambda *s: _rng.normal(s) * 0.05)(B, M, Dm)), 'Wq': _w((lambda *s: _rng.normal(s) * 0.05)(Dm, H, Dh) * Dm ** (-0.5)), 'Wk': _w((lambda *s: _rng.normal(s) * 0.05)(Dm, H, Dh) * Dm ** (-0.5)), 'Wv': _w((lambda *s: _rng.normal(s) * 0.05)(Dm, H, Dh) * Dm ** (-0.5)), 'Wo': _w((lambda *s: _rng.normal(s) * 0.05)(H, Dh, Dm) * (H * Dh) ** (-0.5)), 'seg_len': seg}
    _B_in = _B_setup()
    return {'A_x': _A_in['x'], 'A_wqkv': _A_in['wqkv'], 'A_wo': _A_in['wo'], 'B_x': _B_in['x'], 'B_mem0': _B_in['mem0'], 'B_Wq': _B_in['Wq'], 'B_Wk': _B_in['Wk'], 'B_Wv': _B_in['Wv'], 'B_Wo': _B_in['Wo'], 'B_seg_len': _B_in['seg_len'], 'gate_w': _w((lambda *s: _rng.normal(s) * 0.05)(1024))}

def reference(A_x, A_wqkv, A_wo, B_x, B_mem0, B_Wq, B_Wk, B_Wv, B_Wo, B_seg_len, gate_w):

    def _A_ref(x, wqkv, wo):
        B, S, D = x.shape
        H = 32
        Dh = D // H
        qkv = (lambda x, *d: x.transpose(*d))((x @ wqkv).reshape(B, S, 3, H, Dh), 2, 0, 3, 1, 4)
        q, k, v = (qkv[0], qkv[1], qkv[2])
        scale = Dh ** (-0.5)
        scores = jnp.einsum('bhqd,bhkd->bhqk', q, k) * scale
        p = _softmax(scores, axis=-1)
        o = jnp.einsum('bhqk,bhkd->bhqd', p, v)
        return (lambda x, *d: x.transpose(*d))(o, 0, 2, 1, 3).reshape(B, S, D) @ wo

    def _B_ref(x, mem0, Wq, Wk, Wv, Wo, seg_len):
        B, S, Dm = x.shape
        H, Dh = (Wq.shape[1], Wq.shape[2])
        M = mem0.shape[1]
        scale = Dh ** (-0.5)
        n_seg = S // seg_len
        L = M + seg_len
        idx = jnp.arange(L)
        mask = (idx[:, None] < M) | (idx[:, None] >= idx[None, :])
        mem = mem0
        outs = []
        for s in range(n_seg):
            xs = x[:, s * seg_len:(s + 1) * seg_len, :].copy()
            h = jnp.concatenate([mem, xs], axis=1)
            q = jnp.einsum('btd,dhe->bhte', h, Wq)
            k = jnp.einsum('btd,dhe->bhte', h, Wk)
            v = jnp.einsum('btd,dhe->bhte', h, Wv)
            scores = jnp.einsum('bhqe,bhke->bhqk', q, k) * scale
            scores = jnp.where(mask[None, None], scores, -1000000000.0)
            p = _softmax(scores, axis=-1)
            o = jnp.einsum('bhqk,bhke->bhqe', p, v)
            o = jnp.einsum('bhte,hed->btd', o, Wo)
            mem = o[:, :M, :].copy()
            outs.append(o[:, M:, :])
        return jnp.concatenate(outs, axis=1)
    x = A_x
    g = _sigmoid((x * gate_w).sum(-1, keepdims=True))
    a = _A_ref(x, A_wqkv, A_wo)
    b = _B_ref(x, B_mem0, B_Wq, B_Wk, B_Wv, B_Wo, B_seg_len)
    return g * a + (1 - g) * b
```

```python
import functools
import math

import jax
import jax.numpy as jnp
from jax import lax
import jax.experimental.pallas as pl
import jax.experimental.pallas.tpu as pltpu

F32 = jnp.float32
BF16 = jnp.bfloat16
U32 = jnp.uint32

S = 2048
D = 1024
HA = 32
DA = D // HA
HB = 32
DB = 128
MEM = 8
SEG = 32
LB = SEG + MEM
NSEG = S // SEG

QB = 512
KC = 256
NQ = S // QB
NC = S // KC
CB = 512
RB = 1024

LOG2E = math.log2(math.e)
NN = (((1,), (0,)), ((), ()))
NT = (((1,), (1,)), ((), ()))
TN = (((0,), (0,)), ((), ()))


def _dot(a, b, dims=NN):
    return lax.dot_general(a, b, dims, preferred_element_type=F32)


def _round(x):
    return x.astype(BF16).astype(F32)


def _kernel(xa_hbm, wqkv_hbm, woa_hbm, xb_hbm, mem_ref, wq_hbm, wk_hbm, wv_hbm,
            wob_hbm, gw_ref, out_hbm,
            xa, wqkv, woa, xb, wq, wk, wv, wob,
            qk, vt, ot, s0, s1, m0, m1, ga, omg, hbuf, outv, sems):
    def cp_xa(r):
        return pltpu.make_async_copy(
            xa_hbm.at[pl.ds(r * RB, RB)], xa.at[pl.ds(r * RB, RB)], sems.at[r])

    def cp_wqkv(c):
        return pltpu.make_async_copy(
            wqkv_hbm.at[:, pl.ds(c * CB, CB)], wqkv.at[c], sems.at[2 + c])

    cp_woa = pltpu.make_async_copy(woa_hbm, woa, sems.at[8])
    cp_xb = pltpu.make_async_copy(xb_hbm, xb, sems.at[9])
    cp_wq = pltpu.make_async_copy(wq_hbm, wq.bitcast(BF16), sems.at[10])
    cp_wk = pltpu.make_async_copy(wk_hbm, wk.bitcast(BF16), sems.at[11])
    cp_wv = pltpu.make_async_copy(wv_hbm, wv.bitcast(BF16), sems.at[12])

    def cp_wob(j):
        return pltpu.make_async_copy(
            wob_hbm.at[:, pl.ds(j * 128, 128)], wob.bitcast(BF16).at[j], sems.at[13 + j])

    cp_xa(0).start()
    cp_wqkv(0).start()
    cp_xa(1).start()
    for c in range(1, 6):
        cp_wqkv(c).start()
    cp_woa.start()
    cp_xb.start()
    cp_wq.start()
    cp_wk.start()
    cp_wv.start()
    for j in range(8):
        cp_wob(j).start()

    cp_xa(0).wait()
    cp_xa(1).wait()
    for c in range(6):
        cp_wqkv(c).wait()

    qscale = (DA ** -0.5) * LOG2E
    nrb = S // RB

    def qk_body(i, carry):
        c = i // nrb
        r = i % nrb
        x = xa[pl.ds(pl.multiple_of(r * RB, RB), RB), :]
        y = _dot(x, wqkv[c])
        y = y * jnp.where(c < 2, qscale, 1.0).astype(F32)
        yb = pltpu.bitcast(y.astype(BF16), U32)
        for g in range(CB // 128):
            qk[c * (CB // 128) + g, pl.ds(pl.multiple_of(r * (RB // 2), RB // 2), RB // 2), :] = (
                yb[:, g * 128:(g + 1) * 128])
        return carry

    lax.fori_loop(0, 4 * nrb, qk_body, 0)

    def v_body(i, carry):
        c = i // nrb
        r = i % nrb
        x = xa[pl.ds(pl.multiple_of(r * RB, RB), RB), :]
        y = _dot(x, wqkv[4 + c])
        yt = pltpu.bitcast(y.T.astype(BF16), U32)
        for k in range(RB // KC):
            vt[r * (RB // KC) + k, pl.ds(pl.multiple_of(c * (CB // 2), CB // 2), CB // 2), :] = (
                yt[:, k * KC:(k + 1) * KC])
        return carry

    lax.fori_loop(0, 2 * nrb, v_body, 0)

    lane_grp = lax.broadcasted_iota(jnp.int32, (QB // 2, 128), 1) // DA

    def stage(blk_a, s_w, m_w, blk_b, s_r, m_r):
        if blk_a is not None:
            ha = blk_a // NQ
            qa = blk_a % NQ
            g = ha // 4
            qt = qk[g, pl.ds(pl.multiple_of(qa * (QB // 2), QB // 2), QB // 2), :]
            qm = pltpu.bitcast(jnp.where(lane_grp == ha % 4, qt, jnp.zeros_like(qt)), BF16)
            mrun = None
        if blk_b is not None:
            hb = blk_b // NQ
            qb = blk_b % NQ
            mb = m_r[...]
            l = acc = None
        for c in range(NC):
            if blk_a is not None:
                kc = pltpu.bitcast(qk[8 + g, pl.ds(c * (KC // 2), KC // 2), :], BF16)
                s = _dot(kc, qm, NT)
                s_w[pl.ds(c * KC, KC), :] = s
                mc = jnp.max(s.reshape(KC // 8, 8, QB), axis=0)
                mrun = mc if mrun is None else jnp.maximum(mrun, mc)
            if blk_b is not None:
                sr = s_r[pl.ds(c * KC, KC), :]
                p = jnp.exp2(sr.reshape(KC // 8, 8, QB) - mb[None])
                lc = jnp.sum(p, axis=0)
                l = lc if l is None else l + lc
                pb = p.reshape(KC, QB).astype(BF16)
                v = pltpu.bitcast(
                    vt[c, pl.ds(pl.multiple_of(hb * (DA // 2), DA // 2), DA // 2), :], BF16)
                d = _dot(v, pb)
                acc = d if acc is None else acc + d
        if blk_a is not None:
            m_w[...] = jnp.broadcast_to(jnp.max(mrun, axis=0, keepdims=True), (8, QB))
        if blk_b is not None:
            o = acc / jnp.sum(l, axis=0, keepdims=True)
            ot[qb, pl.ds(pl.multiple_of(hb * (DA // 2), DA // 2), DA // 2), :] = pltpu.bitcast(
                o.astype(BF16), U32)

    nblk = HA * NQ
    stage(0, s0, m0, None, None, None)

    def att_body(i, carry):
        b = 2 * i
        stage(b + 1, s1, m1, b, s0, m0)
        stage(jnp.minimum(b + 2, nblk - 1), s0, m0, b + 1, s1, m1)
        return carry

    lax.fori_loop(0, nblk // 2, att_body, 0)

    cp_woa.wait()

    def a3_body(i, carry):
        rows = pl.ds(pl.multiple_of(i * QB, QB), QB)
        a = _dot(pltpu.bitcast(ot[i], BF16), woa[...], TN)
        z = jnp.sum(xa[rows, :].astype(F32) * gw_ref[...].astype(F32), axis=1, keepdims=True)
        g = jax.nn.sigmoid(z)
        ga[rows, :] = g * a
        omg[rows, :] = jnp.broadcast_to(1.0 - g, (QB, 128))
        return carry

    lax.fori_loop(0, NQ, a3_body, 0)

    cp_wq.wait()
    cp_wk.wait()
    cp_wv.wait()

    def regroup_body(c, carry):
        for w in (wq, wk, wv):
            outs = []
            for j in range(HB // 2):
                a = w[c, pl.ds(j, 8, stride=32), :]
                b = w[c, pl.ds(16 + j, 8, stride=32), :]
                outs.append((a & 0xFFFF) | (b << 16))
                outs.append((a >> 16) | (b & jnp.uint32(0xFFFF0000)))
            for h in range(HB):
                w[c, pl.ds(h * 8, 8), :] = outs[h]
        return carry

    lax.fori_loop(0, D // 16, regroup_body, 0)

    cp_xb.wait()
    for j in range(8):
        cp_wob(j).wait()

    hbuf[pl.ds(SEG, MEM), :] = mem_ref[...].astype(F32)
    row = lax.broadcasted_iota(jnp.int32, (LB, LB), 0)
    col = lax.broadcasted_iota(jnp.int32, (LB, LB), 1)
    mask = (row >= SEG) | (col >= SEG) | (col <= row)
    bscale = DB ** -0.5

    def wtile(w, h):
        return pltpu.bitcast(w[:, pl.ds(h * 8, 8), :].reshape(D // 2, 128), BF16)

    def step(s, carry):
        rows = pl.ds(pl.multiple_of(s * SEG, SEG), SEG)
        hbuf[pl.ds(0, SEG), :] = xb[rows, :].astype(F32)

        def proj(h):
            w = jnp.concatenate([wtile(wq, h), wtile(wk, h), wtile(wv, h)], axis=1)
            y = _dot(hbuf[...], w)
            return _round(y[:, :DB]), y[:, DB:2 * DB].astype(BF16), y[:, 2 * DB:].astype(BF16)

        def scores(q, k):
            sc = jnp.where(mask, _dot(q, k, NT) * bscale, -1000000000.0)
            e = jnp.exp(sc - jnp.max(sc, axis=1, keepdims=True))
            return _round(e), jnp.sum(e, axis=1, keepdims=True)

        def attend(e, l, v):
            return _round(_dot(e, v) / l)

        def oproj(h, o):
            w = jnp.concatenate(
                [pltpu.bitcast(wob[j, pl.ds(h * (DB // 2), DB // 2), :], BF16) for j in range(8)],
                axis=1)
            return _dot(o, w)

        qkv, el, oo = {}, {}, {}
        acc = None
        for t in range(HB + 4):
            if t < HB:
                qkv[t] = proj(t)
            h = t - 1
            if 0 <= h < HB:
                el[h] = scores(qkv[h][0], qkv[h][1])
            h = t - 3
            if 0 <= h < HB:
                oo[h] = attend(*el[h], qkv[h][2])
            h = t - 4
            if 0 <= h < HB:
                y = oproj(h, oo[h])
                acc = y if acc is None else acc + y
        hbuf[pl.ds(SEG, MEM), :] = _round(acc[SEG:])
        res = ga[rows, :] + jnp.tile(omg[rows, :], (1, D // 128)) * acc[:SEG]
        outv[rows, :] = res.astype(BF16)
        pltpu.make_async_copy(outv.at[rows], out_hbm.at[rows], sems.at[21]).start()
        return carry

    lax.fori_loop(0, NSEG, step, 0)
    pltpu.make_async_copy(outv, out_hbm, sems.at[21]).wait()


@jax.jit
def pallas_gated_mix__softmax_full_mha__memory_aug_recurrent_mem_tr__prompt_kernel(
    A_x, A_wqkv, A_wo, B_x, B_mem0, B_Wq, B_Wk, B_Wv, B_Wo, B_seg_len, gate_w,
):
    del B_seg_len
    hbm = pl.BlockSpec(memory_space=pl.ANY)
    vmem = pl.BlockSpec(memory_space=pltpu.VMEM)
    out = pl.pallas_call(
        _kernel,
        out_shape=jax.ShapeDtypeStruct((S, D), BF16),
        in_specs=[hbm, hbm, hbm, hbm, vmem, hbm, hbm, hbm, hbm, vmem],
        out_specs=hbm,
        scratch_shapes=[
            pltpu.VMEM((S, D), BF16),
            pltpu.VMEM((3 * D // CB, D, CB), BF16),
            pltpu.VMEM((D, D), BF16),
            pltpu.VMEM((S, D), BF16),
            pltpu.VMEM((D // 16, 256, 128), U32),
            pltpu.VMEM((D // 16, 256, 128), U32),
            pltpu.VMEM((D // 16, 256, 128), U32),
            pltpu.VMEM((8, HB * DB // 2, 128), U32),
            pltpu.VMEM((16, S // 2, 128), U32),
            pltpu.VMEM((NC, D // 2, KC), U32),
            pltpu.VMEM((NQ, D // 2, QB), U32),
            pltpu.VMEM((S, QB), F32),
            pltpu.VMEM((S, QB), F32),
            pltpu.VMEM((8, QB), F32),
            pltpu.VMEM((8, QB), F32),
            pltpu.VMEM((S, D), F32),
            pltpu.VMEM((S, 128), F32),
            pltpu.VMEM((LB, D), F32),
            pltpu.VMEM((S, D), BF16),
            pltpu.SemaphoreType.DMA((22,)),
        ],
        compiler_params=pltpu.CompilerParams(vmem_limit_bytes=120 * 1024 * 1024),
        name="gated_mix",
    )(
        A_x.reshape(S, D), A_wqkv, A_wo, B_x.reshape(S, D), B_mem0.reshape(MEM, D),
        B_Wq.reshape(D // 16, 16 * HB, DB), B_Wk.reshape(D // 16, 16 * HB, DB),
        B_Wv.reshape(D // 16, 16 * HB, DB), B_Wo.reshape(HB * DB, D), gate_w.reshape(1, D),
    )
    return out.reshape(1, S, D)
```

```python
import math

import jax
import jax.numpy as jnp
from jax import lax
import jax.experimental.pallas as pl
import jax.experimental.pallas.tpu as pltpu

F32 = jnp.float32
BF16 = jnp.bfloat16
U32 = jnp.uint32

S = 2048
D = 1024
HA = 32
DA = D // HA
HB = 32
DB = 128
MEM = 8
SEG = 32
LB = SEG + MEM
NSEG = S // SEG

QB = 512
KC = 128
NQ = S // QB
NC = S // KC
CB = 512
RB = 1024
NSTAGE = HA * NQ // 2

LOG2E = math.log2(math.e)
NN = (((1,), (0,)), ((), ()))
NT = (((1,), (1,)), ((), ()))


def _dot(a, b, dims=NN):
    return lax.dot_general(a, b, dims, preferred_element_type=F32)


def _round(x):
    return x.astype(BF16).astype(F32)


def _kernel(xa_hbm, wqkv_hbm, woa_hbm, xb_hbm, mem_ref, wq_hbm, wk_hbm, wv_hbm,
            wob_hbm, gw_ref, out_hbm,
            xa, wqkv, woa, xb, wb, wob, qk, vt, on, oprev, sbuf, mbuf, ga, omg,
            hbuf, outv, sems, wsems):
    def cp_xa(r):
        return pltpu.make_async_copy(
            xa_hbm.at[pl.ds(r * RB, RB)], xa.at[pl.ds(r * RB, RB)], sems.at[r])

    def cp_wqkv(c):
        return pltpu.make_async_copy(
            wqkv_hbm.at[:, pl.ds(c * CB, CB)], wqkv.at[c], sems.at[2 + c])

    cp_xb = pltpu.make_async_copy(xb_hbm, xb, sems.at[8])

    def cp_woa(j):
        return pltpu.make_async_copy(
            woa_hbm.at[:, pl.ds(j * 128, 128)], woa.bitcast(BF16).at[j], sems.at[9])

    def cp_wob(j):
        return pltpu.make_async_copy(
            wob_hbm.at[:, pl.ds(j * 128, 128)], wob.bitcast(BF16).at[j], sems.at[10])

    def start_wb():
        for i, w in enumerate((wq_hbm, wk_hbm, wv_hbm)):
            w32 = w.bitcast(U32)
            for j in range(HB // 2):
                for c in range(2):
                    pltpu.make_async_copy(
                        w32.at[:, c, j, :], wb.at[i, 2 * j + c], wsems.at[i]).start()

    def wait_wb():
        for i in range(3):
            pltpu.make_async_copy(wb.at[i], wb.at[i], wsems.at[i]).wait()

    cp_xa(0).start()
    cp_wqkv(0).start()

    qscale = (DA ** -0.5) * LOG2E
    nrb = S // RB

    def qk_body(i, carry):
        c = i // nrb
        r = i % nrb

        @pl.when(i == 0)
        def _():
            cp_xa(0).wait()
            cp_wqkv(0).wait()
            cp_xa(1).start()
            cp_wqkv(1).start()

        @pl.when(i == 1)
        def _():
            cp_xa(1).wait()
            for k in range(2, 6):
                cp_wqkv(k).start()

        @pl.when(i == 2)
        def _():
            cp_wqkv(1).wait()

        @pl.when(i == 4)
        def _():
            for k in range(2, 6):
                cp_wqkv(k).wait()
            start_wb()

        x = xa[pl.ds(pl.multiple_of(r * RB, RB), RB), :]
        y = _dot(x, wqkv[c])
        y = y * jnp.where(c < 2, qscale, 1.0).astype(F32)
        yb = pltpu.bitcast(y.astype(BF16), U32)
        for g in range(CB // 128):
            qk[c * (CB // 128) + g, pl.ds(pl.multiple_of(r * (RB // 2), RB // 2), RB // 2), :] = (
                yb[:, g * 128:(g + 1) * 128])
        return carry

    lax.fori_loop(0, 4 * nrb, qk_body, 0)

    def v_body(i, carry):
        c = i // nrb
        r = i % nrb
        x = xa[pl.ds(pl.multiple_of(r * RB, RB), RB), :]
        y = _dot(x, wqkv[4 + c])
        yt = pltpu.bitcast(y.T.astype(BF16), U32)
        for k in range(RB // KC):
            vt[r * (RB // KC) + k, pl.ds(pl.multiple_of(c * (CB // 2), CB // 2), CB // 2), :] = (
                yt[:, k * KC:(k + 1) * KC])
        return carry

    lax.fori_loop(0, 2 * nrb, v_body, 0)

    cp_xb.start()
    for j in range(8):
        cp_woa(j).start()
        cp_wob(j).start()
    wait_wb()

    lane_grp = lax.broadcasted_iota(jnp.int32, (QB // 2, 128), 1) // DA

    def flush_prev(t, par):
        o = oprev[...].T.astype(BF16)
        rows = pl.ds(pl.multiple_of(((t // 2) % NQ) * QB, QB), QB)
        on[t // (2 * NQ), rows, pl.ds(par * 2 * DA, 2 * DA)] = o

    def stage(ta, tb, par):
        qk_parts, pv_parts = [], []
        for j in range(2):
            def make(j):
                st = dict(m=None, l=None, acc=None)

                def qk_part(c):
                    s_w, m_w = sbuf[2 * (1 - par) + j], mbuf[2 * (1 - par) + j]
                    g = ta // (2 * NQ)
                    if c == 0:
                        qa = (ta // 2) % NQ
                        qt = qk[g, pl.ds(pl.multiple_of(qa * (QB // 2), QB // 2), QB // 2), :]
                        st['q'] = pltpu.bitcast(
                            jnp.where(lane_grp == 2 * (1 - par) + j, qt, jnp.zeros_like(qt)), BF16)
                    kc = pltpu.bitcast(qk[8 + g, pl.ds(c * (KC // 2), KC // 2), :], BF16)
                    s = _dot(kc, st['q'], NT)
                    s_w[pl.ds(c * KC, KC), :] = s
                    mc = jnp.max(s.reshape(KC // 8, 8, QB), axis=0)
                    st['m'] = mc if st['m'] is None else jnp.maximum(st['m'], mc)
                    if c == NC - 1:
                        m_w[...] = jnp.broadcast_to(
                            jnp.max(st['m'], axis=0, keepdims=True), (8, QB))

                def pv_part(c):
                    s_r, m_r = sbuf[2 * par + j], mbuf[2 * par + j]
                    if c == 0:
                        st['mb'] = m_r[...]
                    ps = [None] * (KC // 16)
                    for r in reversed(range(KC // 16)):
                        base = c * KC + r * 16
                        p1 = jnp.exp2(s_r[pl.ds(base + 8, 8), :] - st['mb'])
                        p0 = jnp.exp2(s_r[pl.ds(base, 8), :] - st['mb'])
                        st['l'] = p1 if st['l'] is None else st['l'] + p1
                        st['l'] = st['l'] + p0
                        ps[r] = jnp.concatenate([p0, p1], axis=0).astype(BF16)
                    h = (tb // (2 * NQ)) * 4 + 2 * par + j
                    v = pltpu.bitcast(
                        vt[c, pl.ds(pl.multiple_of(h * (DA // 2), DA // 2), DA // 2), :], BF16)
                    d = _dot(v, jnp.concatenate(ps, axis=0))
                    st['acc'] = d if st['acc'] is None else st['acc'] + d
                    if c == NC - 1:
                        oprev[pl.ds(j * DA, DA), :] = (
                            st['acc'] / jnp.sum(st['l'], axis=0, keepdims=True))

                return qk_part, pv_part

            qk_part, pv_part = make(j)
            qk_parts += [(qk_part, c) for c in range(NC)]
            pv_parts += [(pv_part, c) for c in range(NC)]
        for (fq, c), (fp, _) in zip(qk_parts, pv_parts):
            if ta is not None:
                fq(c)
            if tb is not None:
                fp(c)

    def regroup(t):
        per = HB // 2 * 4
        j = t // 4
        rows = pl.ds(pl.multiple_of((t % 4) * 128, 128), 128)
        assert per == NSTAGE
        for i in range(3):
            a = wb[i, 2 * j, rows, :]
            b = wb[i, 2 * j + 1, rows, :]
            wb[i, 2 * j, rows, :] = (a & 0xFFFF) | (b << 16)
            wb[i, 2 * j + 1, rows, :] = (a >> 16) | (b & jnp.uint32(0xFFFF0000))

    stage(0, None, 1)
    oprev[...] = jnp.zeros_like(oprev)

    def att_body(t, carry):
        nxt = jnp.minimum(t + 1, NSTAGE - 1)
        for par in range(2):
            @pl.when(t % 2 == par)
            def _():
                flush_prev(jnp.maximum(t - 1, 0), 1 - par)
                regroup(t)
                stage(nxt, t, par)
        return carry

    lax.fori_loop(0, NSTAGE, att_body, 0)
    flush_prev(NSTAGE - 1, 1)

    cp_xb.wait()
    pltpu.make_async_copy(woa, woa, sems.at[9]).wait()
    pltpu.make_async_copy(wob, wob, sems.at[10]).wait()

    hbuf[pl.ds(SEG, MEM), :] = mem_ref[...].astype(F32)
    row = lax.broadcasted_iota(jnp.int32, (LB, LB), 0)
    col = lax.broadcasted_iota(jnp.int32, (LB, LB), 1)
    mask = (row >= SEG) | (col >= SEG) | (col <= row)
    bscale = DB ** -0.5

    def gate(rows):
        z = jnp.sum(xa[rows, :].astype(F32) * gw_ref[...].astype(F32), axis=1, keepdims=True)
        return jax.nn.sigmoid(z)

    def a_part(rows, g, n0, n1):
        o = jnp.concatenate([on[k, rows, :] for k in range(D // 128)], axis=1)
        w = jnp.concatenate([pltpu.bitcast(woa[j], BF16) for j in range(n0, n1)], axis=1)
        ga[:, pl.ds(n0 * 128, (n1 - n0) * 128)] = g * _dot(o, w)

    g0 = gate(pl.ds(0, SEG))
    a_part(pl.ds(0, SEG), g0, 0, 8)
    omg[...] = jnp.broadcast_to(1.0 - g0, (SEG, 128))

    def step(s, carry):
        rows = pl.ds(pl.multiple_of(s * SEG, SEG), SEG)
        nrows = pl.ds(pl.multiple_of(jnp.minimum(s + 1, NSEG - 1) * SEG, SEG), SEG)
        hbuf[pl.ds(0, SEG), :] = xb[rows, :].astype(F32)
        ga_s = ga[...]
        omg_s = omg[...]
        g = gate(nrows)
        omg[...] = jnp.broadcast_to(1.0 - g, (SEG, 128))

        def proj(h):
            w = jnp.concatenate([pltpu.bitcast(wb[i, h], BF16) for i in range(3)], axis=1)
            y = _dot(hbuf[...], w)
            return _round(y[:, :DB]), y[:, DB:2 * DB].astype(BF16), y[:, 2 * DB:].astype(BF16)

        def scores(q, k):
            sc = jnp.where(mask, _dot(q, k, NT) * bscale, -1000000000.0)
            e = jnp.exp(sc - jnp.max(sc, axis=1, keepdims=True))
            return _round(e), jnp.sum(e, axis=1, keepdims=True)

        def attend(e, l, v):
            return _round(_dot(e, v) / l)

        def oproj(h, o):
            w = jnp.concatenate(
                [pltpu.bitcast(wob[j, pl.ds(h * (DB // 2), DB // 2), :], BF16) for j in range(8)],
                axis=1)
            return _dot(o, w)

        qkv, el, oo = {}, {}, {}
        acc = None
        for t in range(HB + 4):
            if t < HB:
                qkv[t] = proj(t)
            h = t - 1
            if 0 <= h < HB:
                el[h] = scores(qkv[h][0], qkv[h][1])
            h = t - 3
            if 0 <= h < HB:
                oo[h] = attend(*el[h], qkv[h][2])
            h = t - 4
            if 0 <= h < HB:
                y = oproj(h, oo[h])
                acc = y if acc is None else acc + y
            if t >= HB:
                a_part(nrows, g, 2 * (t - HB), 2 * (t - HB) + 2)
        hbuf[pl.ds(SEG, MEM), :] = _round(acc[SEG:])
        res = ga_s + jnp.tile(omg_s, (1, D // 128)) * acc[:SEG]
        outv[rows, :] = res.astype(BF16)
        pltpu.make_async_copy(outv.at[rows], out_hbm.at[rows], sems.at[11]).start()
        return carry

    lax.fori_loop(0, NSEG, step, 0)
    pltpu.make_async_copy(outv, out_hbm, sems.at[11]).wait()


@jax.jit
def pallas_gated_mix__softmax_full_mha__memory_aug_recurrent_mem_tr__prompt_kernel(
    A_x, A_wqkv, A_wo, B_x, B_mem0, B_Wq, B_Wk, B_Wv, B_Wo, B_seg_len, gate_w,
):
    del B_seg_len
    hbm = pl.BlockSpec(memory_space=pl.ANY)
    vmem = pl.BlockSpec(memory_space=pltpu.VMEM)
    split_d = (D // 2, 2, HB, DB)
    out = pl.pallas_call(
        _kernel,
        out_shape=jax.ShapeDtypeStruct((S, D), BF16),
        in_specs=[hbm, hbm, hbm, hbm, vmem, hbm, hbm, hbm, hbm, vmem],
        out_specs=hbm,
        scratch_shapes=[
            pltpu.VMEM((S, D), BF16),
            pltpu.VMEM((3 * D // CB, D, CB), BF16),
            pltpu.VMEM((8, D // 2, 128), U32),
            pltpu.VMEM((S, D), BF16),
            pltpu.VMEM((3, HB, D // 2, 128), U32),
            pltpu.VMEM((8, HB * DB // 2, 128), U32),
            pltpu.VMEM((16, S // 2, 128), U32),
            pltpu.VMEM((NC, D // 2, KC), U32),
            pltpu.VMEM((8, S, 128), BF16),
            pltpu.VMEM((2 * DA, QB), F32),
            [pltpu.VMEM((S, QB), F32) for _ in range(4)],
            [pltpu.VMEM((8, QB), F32) for _ in range(4)],
            pltpu.VMEM((SEG, D), F32),
            pltpu.VMEM((SEG, 128), F32),
            pltpu.VMEM((LB, D), F32),
            pltpu.VMEM((S, D), BF16),
            pltpu.SemaphoreType.DMA((12,)),
            pltpu.SemaphoreType.DMA((3,)),
        ],
        compiler_params=pltpu.CompilerParams(vmem_limit_bytes=120 * 1024 * 1024),
        name="gated_mix",
    )(
        A_x.reshape(S, D), A_wqkv, A_wo, B_x.reshape(S, D), B_mem0.reshape(MEM, D),
        B_Wq.reshape(split_d), B_Wk.reshape(split_d), B_Wv.reshape(split_d),
        B_Wo.reshape(HB * DB, D), gate_w.reshape(1, D),
    )
    return out.reshape(1, S, D)
```

```python
import math

import jax
import jax.numpy as jnp
from jax import lax
import jax.experimental.pallas as pl
import jax.experimental.pallas.tpu as pltpu

F32 = jnp.float32
BF16 = jnp.bfloat16
U32 = jnp.uint32

S = 2048
D = 1024
HA = 32
DA = D // HA
HB = 32
DB = 128
MEM = 8
SEG = 32
LB = SEG + MEM
NSEG = S // SEG

QB = 512
KC = 128
NQ = S // QB
NC = S // KC
CB = 512
RB = 1024
NSTAGE = HA * NQ // 2

LOG2E = math.log2(math.e)
NN = (((1,), (0,)), ((), ()))
NT = (((1,), (1,)), ((), ()))


def _dot(a, b, dims=NN):
    return lax.dot_general(a, b, dims, preferred_element_type=F32)


def _round(x):
    return x.astype(BF16).astype(F32)


def _kernel(xa_hbm, wqkv_hbm, woa_hbm, xb_hbm, mem_ref, wq_hbm, wk_hbm, wv_hbm,
            wob_hbm, gw_ref, out_hbm,
            xa, wqkv, woa, xb, wb, wob, qk, vt, on, oprev, sbuf, mbuf, ga, omg,
            hbuf, outv, sems, wsems):
    def cp_xa(r):
        return pltpu.make_async_copy(
            xa_hbm.at[pl.ds(r * RB, RB)], xa.at[pl.ds(r * RB, RB)], sems.at[r])

    def cp_wqkv(c):
        return pltpu.make_async_copy(
            wqkv_hbm.at[:, pl.ds(c * CB, CB)], wqkv.at[c], sems.at[2 + c])

    cp_xb = pltpu.make_async_copy(xb_hbm, xb, sems.at[8])

    def cp_woa(j):
        return pltpu.make_async_copy(
            woa_hbm.at[:, pl.ds(j * 128, 128)], woa.bitcast(BF16).at[j], sems.at[9])

    def cp_wob(j):
        return pltpu.make_async_copy(
            wob_hbm.at[:, pl.ds(j * 128, 128)], wob.bitcast(BF16).at[j], sems.at[10])

    def start_wb(part):
        i, c = divmod(part, 2)
        w32 = (wq_hbm, wk_hbm, wv_hbm)[i].bitcast(U32)
        for j in range(HB // 2):
            pltpu.make_async_copy(
                w32.at[:, c, j, :], wb.at[i, 2 * j + c], wsems.at[i]).start()

    def wait_wb():
        for i in range(3):
            pltpu.make_async_copy(wb.at[i], wb.at[i], wsems.at[i]).wait()

    cp_xa(0).start()
    cp_wqkv(0).start()

    qscale = (DA ** -0.5) * LOG2E
    nrb = S // RB

    def qk_body(i, carry):
        c = i // nrb
        r = i % nrb

        @pl.when(i == 0)
        def _():
            cp_xa(0).wait()
            cp_wqkv(0).wait()
            cp_xa(1).start()
            cp_wqkv(1).start()

        @pl.when(i == 1)
        def _():
            cp_xa(1).wait()
            for k in range(2, 6):
                cp_wqkv(k).start()

        @pl.when(i == 2)
        def _():
            cp_wqkv(1).wait()

        @pl.when(i == 4)
        def _():
            for k in range(2, 6):
                cp_wqkv(k).wait()

        for k in range(4):
            @pl.when(i == 4 + k)
            def _():
                start_wb(k)

        x = xa[pl.ds(pl.multiple_of(r * RB, RB), RB), :]
        y = _dot(x, wqkv[c])
        y = y * jnp.where(c < 2, qscale, 1.0).astype(F32)
        yb = pltpu.bitcast(y.astype(BF16), U32)
        for g in range(CB // 128):
            qk[c * (CB // 128) + g, pl.ds(pl.multiple_of(r * (RB // 2), RB // 2), RB // 2), :] = (
                yb[:, g * 128:(g + 1) * 128])
        return carry

    lax.fori_loop(0, 4 * nrb, qk_body, 0)

    def v_body(i, carry):
        c = i // nrb
        r = i % nrb
        for k in range(2):
            @pl.when(i == k)
            def _():
                start_wb(4 + k)

        x = xa[pl.ds(pl.multiple_of(r * RB, RB), RB), :]
        y = _dot(x, wqkv[4 + c])
        yt = pltpu.bitcast(y.T.astype(BF16), U32)
        for k in range(RB // KC):
            vt[r * (RB // KC) + k, pl.ds(pl.multiple_of(c * (CB // 2), CB // 2), CB // 2), :] = (
                yt[:, k * KC:(k + 1) * KC])
        return carry

    lax.fori_loop(0, 2 * nrb, v_body, 0)

    cp_xb.start()
    for j in range(8):
        cp_woa(j).start()
        cp_wob(j).start()
    wait_wb()

    lane_grp = lax.broadcasted_iota(jnp.int32, (QB // 2, 128), 1) // DA

    def flush_prev(t, par):
        o = oprev[...].T.astype(BF16)
        rows = pl.ds(pl.multiple_of(((t // 2) % NQ) * QB, QB), QB)
        on[t // (2 * NQ), rows, pl.ds(par * 2 * DA, 2 * DA)] = o

    def stage(ta, tb, par):
        qk_parts, pv_parts = [], []
        for j in range(2):
            def make(j):
                st = dict(m=None, l=None, acc=None)

                def qk_part(c):
                    s_w, m_w = sbuf[2 * (1 - par) + j], mbuf[2 * (1 - par) + j]
                    g = ta // (2 * NQ)
                    if c == 0:
                        qa = (ta // 2) % NQ
                        qt = qk[g, pl.ds(pl.multiple_of(qa * (QB // 2), QB // 2), QB // 2), :]
                        st['q'] = pltpu.bitcast(
                            jnp.where(lane_grp == 2 * (1 - par) + j, qt, jnp.zeros_like(qt)), BF16)
                    kc = pltpu.bitcast(qk[8 + g, pl.ds(c * (KC // 2), KC // 2), :], BF16)
                    s = _dot(kc, st['q'], NT)
                    s_w[pl.ds(c * KC, KC), :] = s
                    mc = jnp.max(s.reshape(KC // 8, 8, QB), axis=0)
                    st['m'] = mc if st['m'] is None else jnp.maximum(st['m'], mc)
                    if c == NC - 1:
                        m_w[...] = jnp.broadcast_to(
                            jnp.max(st['m'], axis=0, keepdims=True), (8, QB))

                def pv_part(c):
                    s_r, m_r = sbuf[2 * par + j], mbuf[2 * par + j]
                    if c == 0:
                        st['mb'] = m_r[...]
                    ps = [None] * (KC // 16)
                    for r in reversed(range(KC // 16)):
                        base = c * KC + r * 16
                        p1 = jnp.exp2(s_r[pl.ds(base + 8, 8), :] - st['mb'])
                        p0 = jnp.exp2(s_r[pl.ds(base, 8), :] - st['mb'])
                        st['l'] = p1 if st['l'] is None else st['l'] + p1
                        st['l'] = st['l'] + p0
                        ps[r] = jnp.concatenate([p0, p1], axis=0).astype(BF16)
                    h = (tb // (2 * NQ)) * 4 + 2 * par + j
                    v = pltpu.bitcast(
                        vt[c, pl.ds(pl.multiple_of(h * (DA // 2), DA // 2), DA // 2), :], BF16)
                    d = _dot(v, jnp.concatenate(ps, axis=0))
                    st['acc'] = d if st['acc'] is None else st['acc'] + d
                    if c == NC - 1:
                        oprev[pl.ds(j * DA, DA), :] = (
                            st['acc'] / jnp.sum(st['l'], axis=0, keepdims=True))

                return qk_part, pv_part

            qk_part, pv_part = make(j)
            qk_parts += [(qk_part, c) for c in range(NC)]
            pv_parts += [(pv_part, c) for c in range(NC)]
        for (fq, c), (fp, _) in zip(qk_parts, pv_parts):
            if ta is not None:
                fq(c)
            if tb is not None:
                fp(c)

    def regroup(t):
        per = HB // 2 * 4
        j = t // 4
        rows = pl.ds(pl.multiple_of((t % 4) * 128, 128), 128)
        assert per == NSTAGE
        for i in range(3):
            a = wb[i, 2 * j, rows, :]
            b = wb[i, 2 * j + 1, rows, :]
            wb[i, 2 * j, rows, :] = (a & 0xFFFF) | (b << 16)
            wb[i, 2 * j + 1, rows, :] = (a >> 16) | (b & jnp.uint32(0xFFFF0000))

    stage(0, None, 1)
    oprev[...] = jnp.zeros_like(oprev)

    def att_body(t, carry):
        nxt = jnp.minimum(t + 1, NSTAGE - 1)
        for par in range(2):
            @pl.when(t % 2 == par)
            def _():
                flush_prev(jnp.maximum(t - 1, 0), 1 - par)
                regroup(t)
                stage(nxt, t, par)
        return carry

    lax.fori_loop(0, NSTAGE, att_body, 0)
    flush_prev(NSTAGE - 1, 1)

    cp_xb.wait()
    pltpu.make_async_copy(woa, woa, sems.at[9]).wait()
    pltpu.make_async_copy(wob, wob, sems.at[10]).wait()

    hbuf[pl.ds(SEG, MEM), :] = mem_ref[...].astype(F32)
    row = lax.broadcasted_iota(jnp.int32, (LB, LB), 0)
    col = lax.broadcasted_iota(jnp.int32, (LB, LB), 1)
    mask = (row >= SEG) | (col >= SEG) | (col <= row)
    bscale = DB ** -0.5

    def gate(rows):
        z = jnp.sum(xa[rows, :].astype(F32) * gw_ref[...].astype(F32), axis=1, keepdims=True)
        return jax.nn.sigmoid(z)

    def a_part(rows, g, n0, n1):
        o = jnp.concatenate([on[k, rows, :] for k in range(D // 128)], axis=1)
        w = jnp.concatenate([pltpu.bitcast(woa[j], BF16) for j in range(n0, n1)], axis=1)
        ga[:, pl.ds(n0 * 128, (n1 - n0) * 128)] = g * _dot(o, w)

    g0 = gate(pl.ds(0, SEG))
    a_part(pl.ds(0, SEG), g0, 0, 8)
    omg[...] = jnp.broadcast_to(1.0 - g0, (SEG, 128))

    def step(s, carry):
        rows = pl.ds(pl.multiple_of(s * SEG, SEG), SEG)
        nrows = pl.ds(pl.multiple_of(jnp.minimum(s + 1, NSEG - 1) * SEG, SEG), SEG)
        hbuf[pl.ds(0, SEG), :] = xb[rows, :].astype(F32)
        ga_s = ga[...]
        omg_s = omg[...]
        g = gate(nrows)
        omg[...] = jnp.broadcast_to(1.0 - g, (SEG, 128))

        def proj(h):
            w = jnp.concatenate([pltpu.bitcast(wb[i, h], BF16) for i in range(3)], axis=1)
            y = _dot(hbuf[...], w)
            return _round(y[:, :DB]), y[:, DB:2 * DB].astype(BF16), y[:, 2 * DB:].astype(BF16)

        def scores(q, k):
            sc = jnp.where(mask, _dot(q, k, NT) * bscale, -1000000000.0)
            e = jnp.exp(sc - jnp.max(sc, axis=1, keepdims=True))
            return _round(e), jnp.sum(e, axis=1, keepdims=True)

        def attend(e, l, v):
            return _round(_dot(e, v) / l)

        def oproj(h, o):
            w = jnp.concatenate(
                [pltpu.bitcast(wob[j, pl.ds(h * (DB // 2), DB // 2), :], BF16) for j in range(8)],
                axis=1)
            return _dot(o, w)

        qkv, el, oo = {}, {}, {}
        acc = None
        for t in range(HB + 4):
            if t < HB:
                qkv[t] = proj(t)
            h = t - 1
            if 0 <= h < HB:
                el[h] = scores(qkv[h][0], qkv[h][1])
            h = t - 3
            if 0 <= h < HB:
                oo[h] = attend(*el[h], qkv[h][2])
            h = t - 4
            if 0 <= h < HB:
                y = oproj(h, oo[h])
                acc = y if acc is None else acc + y
            if t >= HB:
                a_part(nrows, g, 2 * (t - HB), 2 * (t - HB) + 2)
        hbuf[pl.ds(SEG, MEM), :] = _round(acc[SEG:])
        res = ga_s + jnp.tile(omg_s, (1, D // 128)) * acc[:SEG]
        outv[rows, :] = res.astype(BF16)
        pltpu.make_async_copy(outv.at[rows], out_hbm.at[rows], sems.at[11]).start()
        return carry

    lax.fori_loop(0, NSEG, step, 0)
    pltpu.make_async_copy(outv, out_hbm, sems.at[11]).wait()


@jax.jit
def pallas_gated_mix__softmax_full_mha__memory_aug_recurrent_mem_tr__prompt_kernel(
    A_x, A_wqkv, A_wo, B_x, B_mem0, B_Wq, B_Wk, B_Wv, B_Wo, B_seg_len, gate_w,
):
    del B_seg_len
    hbm = pl.BlockSpec(memory_space=pl.ANY)
    vmem = pl.BlockSpec(memory_space=pltpu.VMEM)
    split_d = (D // 2, 2, HB, DB)
    out = pl.pallas_call(
        _kernel,
        out_shape=jax.ShapeDtypeStruct((S, D), BF16),
        in_specs=[hbm, hbm, hbm, hbm, vmem, hbm, hbm, hbm, hbm, vmem],
        out_specs=hbm,
        scratch_shapes=[
            pltpu.VMEM((S, D), BF16),
            pltpu.VMEM((3 * D // CB, D, CB), BF16),
            pltpu.VMEM((8, D // 2, 128), U32),
            pltpu.VMEM((S, D), BF16),
            pltpu.VMEM((3, HB, D // 2, 128), U32),
            pltpu.VMEM((8, HB * DB // 2, 128), U32),
            pltpu.VMEM((16, S // 2, 128), U32),
            pltpu.VMEM((NC, D // 2, KC), U32),
            pltpu.VMEM((8, S, 128), BF16),
            pltpu.VMEM((2 * DA, QB), F32),
            [pltpu.VMEM((S, QB), F32) for _ in range(4)],
            [pltpu.VMEM((8, QB), F32) for _ in range(4)],
            pltpu.VMEM((SEG, D), F32),
            pltpu.VMEM((SEG, 128), F32),
            pltpu.VMEM((LB, D), F32),
            pltpu.VMEM((S, D), BF16),
            pltpu.SemaphoreType.DMA((12,)),
            pltpu.SemaphoreType.DMA((3,)),
        ],
        compiler_params=pltpu.CompilerParams(vmem_limit_bytes=120 * 1024 * 1024),
        name="gated_mix",
    )(
        A_x.reshape(S, D), A_wqkv, A_wo, B_x.reshape(S, D), B_mem0.reshape(MEM, D),
        B_Wq.reshape(split_d), B_Wk.reshape(split_d), B_Wv.reshape(split_d),
        B_Wo.reshape(HB * DB, D), gate_w.reshape(1, D),
    )
    return out.reshape(1, S, D)
```

```python
import math
import os

import jax
import jax.numpy as jnp
from jax import lax
import jax.experimental.pallas as pl
import jax.experimental.pallas.tpu as pltpu

F32 = jnp.float32
BF16 = jnp.bfloat16
U32 = jnp.uint32

S = 2048
D = 1024
HA = 32
DA = D // HA
HB = 32
DB = 128
MEM = 8
SEG = 32
LB = SEG + MEM
NSEG = S // SEG

QB = 512
KC = 128
NQ = S // QB
NC = S // KC
CB = 512
RB = 1024
NSTAGE = HA * NQ // 2
OB = 512

SHIFT = int(os.environ.get("SHIFT", 4))
POS = int(os.environ.get("POS", 0))

LOG2E = math.log2(math.e)
NN = (((1,), (0,)), ((), ()))
NT = (((1,), (1,)), ((), ()))
TN = (((0,), (0,)), ((), ()))


def _dot(a, b, dims=NN):
    return lax.dot_general(a, b, dims, preferred_element_type=F32)


def _round(x):
    return x.astype(BF16).astype(F32)


def _kernel(xa_hbm, wqkv_hbm, woa_hbm, xb_hbm, mem_ref, wq_hbm, wk_hbm, wv_hbm,
            wob_hbm, gw_ref, out_hbm,
            xa, wqkv, woa, xb, wb, wob, qk, vt, ot, sbuf, mbuf, bout,
            hbuf, outv, sems, wsems):
    def cp_xa(r):
        return pltpu.make_async_copy(
            xa_hbm.at[pl.ds(r * RB, RB)], xa.at[pl.ds(r * RB, RB)], sems.at[r])

    def cp_wqkv(c):
        return pltpu.make_async_copy(
            wqkv_hbm.at[:, pl.ds(c * CB, CB)], wqkv.at[c], sems.at[2 + c])

    cp_xb = pltpu.make_async_copy(xb_hbm, xb, sems.at[8])
    cp_woa = pltpu.make_async_copy(woa_hbm, woa, sems.at[9])

    def cp_wob(j):
        return pltpu.make_async_copy(
            wob_hbm.at[:, pl.ds(j * 128, 128)], wob.bitcast(BF16).at[j], sems.at[10])

    def start_wb(part):
        for n in range(16 * part, 16 * part + 16):
            j, i, c = n // 6, (n // 2) % 3, n % 2
            w32 = (wq_hbm, wk_hbm, wv_hbm)[i].bitcast(U32)
            pltpu.make_async_copy(
                w32.at[:, c, j, :], wb.at[j, i, c], wsems.at[j // 4]).start()

    cp_xa(0).start()
    cp_wqkv(0).start()

    qscale = (DA ** -0.5) * LOG2E
    nrb = S // RB

    def qk_body(i, carry):
        c = i // nrb
        r = i % nrb

        @pl.when(i == 0)
        def _():
            cp_xa(0).wait()
            cp_wqkv(0).wait()
            cp_xa(1).start()
            cp_wqkv(1).start()

        @pl.when(i == 1)
        def _():
            cp_xa(1).wait()
            for k in range(2, 6):
                cp_wqkv(k).start()

        @pl.when(i == 2)
        def _():
            cp_wqkv(1).wait()

        @pl.when(i == 4)
        def _():
            for k in range(2, 6):
                cp_wqkv(k).wait()

        for k in range(6):
            @pl.when(i == 2 + k)
            def _():
                start_wb(k)

        x = xa[pl.ds(pl.multiple_of(r * RB, RB), RB), :]
        y = _dot(x, wqkv[c])
        y = y * jnp.where(c < 2, qscale, 1.0).astype(F32)
        yb = pltpu.bitcast(y.astype(BF16), U32)
        for g in range(CB // 128):
            qk[c * (CB // 128) + g, pl.ds(pl.multiple_of(r * (RB // 2), RB // 2), RB // 2), :] = (
                yb[:, g * 128:(g + 1) * 128])
        return carry

    lax.fori_loop(0, 4 * nrb, qk_body, 0)

    def v_body(i, carry):
        c = i // nrb
        r = i % nrb

        @pl.when(i == 0)
        def _():
            for j in range(8):
                cp_wob(j).start()

        @pl.when(i == 1)
        def _():
            cp_xb.start()

        @pl.when(i == 2)
        def _():
            cp_woa.start()

        quarter = wb.at[pl.ds(4 * i, 4)]
        pltpu.make_async_copy(quarter, quarter, wsems.at[i]).wait()

        x = xa[pl.ds(pl.multiple_of(r * RB, RB), RB), :]
        y = _dot(x, wqkv[4 + c])
        yt = pltpu.bitcast(y.T.astype(BF16), U32)
        for k in range(RB // KC):
            vt[r * (RB // KC) + k, pl.ds(pl.multiple_of(c * (CB // 2), CB // 2), CB // 2), :] = (
                yt[:, k * KC:(k + 1) * KC])
        for j in range(4):
            for m in range(3):
                a = wb[4 * i + j, m, 0]
                b = wb[4 * i + j, m, 1]
                wb[4 * i + j, m, 0] = (a & 0xFFFF) | (b << 16)
                wb[4 * i + j, m, 1] = (a >> 16) | (b & jnp.uint32(0xFFFF0000))
        return carry

    lax.fori_loop(0, 2 * nrb, v_body, 0)

    lane_grp = lax.broadcasted_iota(jnp.int32, (QB // 2, 128), 1) // DA

    def stage_parts(ta, tb, par):
        qk_parts, pv_parts = [], []
        for j in range(2):
            def make(j):
                st = dict(m=None, l=None, acc=None)

                def qk_part(c):
                    s_w, m_w = sbuf[2 * (1 - par) + j], mbuf[2 * (1 - par) + j]
                    g = ta // (2 * NQ)
                    if c == 0:
                        qa = (ta // 2) % NQ
                        qt = qk[g, pl.ds(pl.multiple_of(qa * (QB // 2), QB // 2), QB // 2), :]
                        st['q'] = pltpu.bitcast(
                            jnp.where(lane_grp == 2 * (1 - par) + j, qt, jnp.zeros_like(qt)), BF16)
                    kc = pltpu.bitcast(qk[8 + g, pl.ds(c * (KC // 2), KC // 2), :], BF16)
                    s = _dot(kc, st['q'], NT)
                    s_w[pl.ds(c * KC, KC), :] = s
                    mc = jnp.max(s.reshape(KC // 8, 8, QB), axis=0)
                    st['m'] = mc if st['m'] is None else jnp.maximum(st['m'], mc)
                    if c == NC - 1:
                        m_w[...] = jnp.broadcast_to(
                            jnp.max(st['m'], axis=0, keepdims=True), (8, QB))

                def pv_part(c):
                    s_r, m_r = sbuf[2 * par + j], mbuf[2 * par + j]
                    if c == 0:
                        st['mb'] = m_r[...]
                    ps = [None] * (KC // 16)
                    for r in reversed(range(KC // 16)):
                        base = c * KC + r * 16
                        p1 = jnp.exp2(s_r[pl.ds(base + 8, 8), :] - st['mb'])
                        p0 = jnp.exp2(s_r[pl.ds(base, 8), :] - st['mb'])
                        st['l'] = p1 if st['l'] is None else st['l'] + p1
                        st['l'] = st['l'] + p0
                        ps[r] = jnp.concatenate([p0, p1], axis=0).astype(BF16)
                    h = (tb // (2 * NQ)) * 4 + 2 * par + j
                    hrows = pl.ds(pl.multiple_of(h * (DA // 2), DA // 2), DA // 2)
                    v = pltpu.bitcast(vt[c, hrows, :], BF16)
                    d = _dot(v, jnp.concatenate(ps, axis=0))
                    st['acc'] = d if st['acc'] is None else st['acc'] + d
                    if c == NC - 1:
                        o = st['acc'] / jnp.sum(st['l'], axis=0, keepdims=True)
                        ot[(tb // 2) % NQ, hrows, :] = pltpu.bitcast(o.astype(BF16), U32)

                return qk_part, pv_part

            qk_part, pv_part = make(j)
            qk_parts += [(qk_part, c) for c in range(NC)]
            pv_parts += [(pv_part, c) for c in range(NC)]
        return qk_parts, pv_parts

    for f, c in stage_parts(0, None, 1)[0]:
        f(c)

    cp_xb.wait()
    pltpu.make_async_copy(wob, wob, sems.at[10]).wait()

    hbuf[pl.ds(SEG, MEM), :] = mem_ref[...].astype(F32)
    row = lax.broadcasted_iota(jnp.int32, (LB, LB), 0)
    col = lax.broadcasted_iota(jnp.int32, (LB, LB), 1)
    mask = (row >= SEG) | (col >= SEG) | (col <= row)
    bscale = DB ** -0.5

    def step(s, par):
        rows = pl.ds(pl.multiple_of(s * SEG, SEG), SEG)
        hbuf[pl.ds(0, SEG), :] = xb[rows, :].astype(F32)
        qk_parts, pv_parts = stage_parts(jnp.minimum(s + 1, NSTAGE - 1), s, par)

        def proj(h):
            w = jnp.concatenate(
                [pltpu.bitcast(wb[h // 2, i, h % 2], BF16) for i in range(3)], axis=1)
            y = _dot(hbuf[...], w)
            return _round(y[:, :DB]), y[:, DB:2 * DB].astype(BF16), y[:, 2 * DB:].astype(BF16)

        def scores(q, k):
            sc = jnp.where(mask, _dot(q, k, NT) * bscale, -1000000000.0)
            e = jnp.exp(sc - jnp.max(sc, axis=1, keepdims=True))
            return _round(e), jnp.sum(e, axis=1, keepdims=True)

        def attend(e, l, v):
            return _round(_dot(e, v) / l)

        def oproj(h, o):
            w = jnp.concatenate(
                [pltpu.bitcast(wob[j, pl.ds(h * (DB // 2), DB // 2), :], BF16) for j in range(8)],
                axis=1)
            return _dot(o, w)

        def att(parts, t):
            if 0 <= t - SHIFT < len(parts):
                f, c = parts[t - SHIFT]
                f(c)

        qkv, el, oo = {}, {}, {}
        acc = None
        for t in range(HB + max(4, SHIFT)):
            if POS == 0:
                att(qk_parts, t)
                att(pv_parts, t)
            if POS == 1:
                att(qk_parts, t)
            if t < HB:
                qkv[t] = proj(t)
            if POS == 1:
                att(pv_parts, t)
            h = t - 1
            if 0 <= h < HB:
                el[h] = scores(qkv[h][0], qkv[h][1])
            h = t - 3
            if 0 <= h < HB:
                oo[h] = attend(*el[h], qkv[h][2])
            h = t - 4
            if 0 <= h < HB:
                y = oproj(h, oo[h])
                acc = y if acc is None else acc + y
            if POS == 2:
                att(qk_parts, t)
                att(pv_parts, t)
        hbuf[pl.ds(SEG, MEM), :] = _round(acc[SEG:])
        bout[rows, :] = acc[:SEG]

    def step_body(s, carry):
        for par in range(2):
            @pl.when(s % 2 == par)
            def _():
                step(s, par)
        return carry

    lax.fori_loop(0, NSEG, step_body, 0)

    cp_woa.wait()

    def out_body(i, carry):
        rows = pl.ds(pl.multiple_of(i * OB, OB), OB)
        a = _dot(pltpu.bitcast(ot[i], BF16), woa[...], TN)
        z = jnp.sum(xa[rows, :].astype(F32) * gw_ref[...].astype(F32), axis=1, keepdims=True)
        g = jax.nn.sigmoid(z)
        outv[rows, :] = (g * a + (1.0 - g) * bout[rows, :]).astype(BF16)
        pltpu.make_async_copy(outv.at[rows], out_hbm.at[rows], sems.at[11]).start()
        return carry

    lax.fori_loop(0, S // OB, out_body, 0)
    pltpu.make_async_copy(outv, out_hbm, sems.at[11]).wait()


@jax.jit
def pallas_gated_mix__softmax_full_mha__memory_aug_recurrent_mem_tr__prompt_kernel(
    A_x, A_wqkv, A_wo, B_x, B_mem0, B_Wq, B_Wk, B_Wv, B_Wo, B_seg_len, gate_w,
):
    del B_seg_len
    hbm = pl.BlockSpec(memory_space=pl.ANY)
    vmem = pl.BlockSpec(memory_space=pltpu.VMEM)
    split_d = (D // 2, 2, HB, DB)
    out = pl.pallas_call(
        _kernel,
        out_shape=jax.ShapeDtypeStruct((S, D), BF16),
        in_specs=[hbm, hbm, hbm, hbm, vmem, hbm, hbm, hbm, hbm, vmem],
        out_specs=hbm,
        scratch_shapes=[
            pltpu.VMEM((S, D), BF16),
            pltpu.VMEM((3 * D // CB, D, CB), BF16),
            pltpu.VMEM((D, D), BF16),
            pltpu.VMEM((S, D), BF16),
            pltpu.VMEM((HB // 2, 3, 2, D // 2, 128), U32),
            pltpu.VMEM((8, HB * DB // 2, 128), U32),
            pltpu.VMEM((16, S // 2, 128), U32),
            pltpu.VMEM((NC, D // 2, KC), U32),
            pltpu.VMEM((NQ, D // 2, QB), U32),
            [pltpu.VMEM((S, QB), F32) for _ in range(4)],
            [pltpu.VMEM((8, QB), F32) for _ in range(4)],
            pltpu.VMEM((S, D), F32),
            pltpu.VMEM((LB, D), F32),
            pltpu.VMEM((S, D), BF16),
            pltpu.SemaphoreType.DMA((12,)),
            pltpu.SemaphoreType.DMA((4,)),
        ],
        compiler_params=pltpu.CompilerParams(vmem_limit_bytes=120 * 1024 * 1024),
        name="gated_mix",
    )(
        A_x.reshape(S, D), A_wqkv, A_wo, B_x.reshape(S, D), B_mem0.reshape(MEM, D),
        B_Wq.reshape(split_d), B_Wk.reshape(split_d), B_Wv.reshape(split_d),
        B_Wo.reshape(HB * DB, D), gate_w.reshape(1, D),
    )
    return out.reshape(1, S, D)
```

```python
import math

import jax
import jax.numpy as jnp
from jax import lax
import jax.experimental.pallas as pl
import jax.experimental.pallas.tpu as pltpu

F32 = jnp.float32
BF16 = jnp.bfloat16
U32 = jnp.uint32

S = 2048
D = 1024
HA = 32
DA = D // HA
HB = 32
DB = 128
MEM = 8
SEG = 32
LB = SEG + MEM
NSEG = S // SEG

QB = 512
KC = 128
NQ = S // QB
NC = S // KC
CB = 512
RB = 1024
SB = 256
NPC = 192

LOG2E = math.log2(math.e)
NN = (((1,), (0,)), ((), ()))
NT = (((1,), (1,)), ((), ()))


def _dot(a, b, dims=NN):
    return lax.dot_general(a, b, dims, preferred_element_type=F32)


def _round(x):
    return x.astype(BF16).astype(F32)


def _kernel(xa_hbm, wqkv_hbm, woa_hbm, xb_hbm, mem_ref, wq_hbm, wk_hbm, wv_hbm,
            wob_hbm, gw_ref, out_hbm,
            xa, wqkv, woa, xb, wb, wob, qk, vt, ot, on, sbuf, mbuf, bout, gate,
            hbuf, outv, zero, sems, wsems):
    def cp_xa(r0, n, sem):
        return pltpu.make_async_copy(
            xa_hbm.at[pl.ds(r0, n)], xa.at[pl.ds(r0, n)], sems.at[sem])

    def cp_wqkv(c):
        return pltpu.make_async_copy(
            wqkv_hbm.at[:, pl.ds(c * CB, CB)], wqkv.at[c], sems.at[5 + c])

    cp_xb = pltpu.make_async_copy(xb_hbm, xb, sems.at[11])
    cp_woa = pltpu.make_async_copy(woa_hbm, woa, sems.at[12])

    def cp_wob(j):
        return pltpu.make_async_copy(
            wob_hbm.at[:, pl.ds(j * 128, 128)], wob.bitcast(BF16).at[j], sems.at[13])

    def start_wb(part):
        for n in range(16 * part, 16 * part + 16):
            j, i, c = n // 6, (n // 2) % 3, n % 2
            w32 = (wq_hbm, wk_hbm, wv_hbm)[i].bitcast(U32)
            pltpu.make_async_copy(
                w32.at[:, c, j, :], wb.at[j, i, c], wsems.at[j // 4]).start()

    cp_wqkv(0).start()
    cp_xa(0, SB, 0).start()

    qscale = (DA ** -0.5) * LOG2E
    nrb = S // RB

    def qk_block(c, r0, n):
        x = xa[pl.ds(r0, n), :]
        y = _dot(x, wqkv[c])
        y = (y * jnp.where(c < 2, qscale, 1.0).astype(F32)).astype(BF16)
        for g in range(CB // 128):
            qk[c * (CB // 128) + g, pl.ds(r0, n), :] = y[:, g * 128:(g + 1) * 128]

    cp_wqkv(0).wait()

    def first_body(i, carry):
        r0 = pl.multiple_of(i * SB, SB)
        cp_xa(r0, SB, i).wait()

        @pl.when(i == 0)
        def _():
            for k in range(1, RB // SB):
                cp_xa(k * SB, SB, k).start()

        @pl.when(i == 1)
        def _():
            cp_xa(RB, S - RB, 4).start()
            cp_wqkv(1).start()

        qk_block(0, r0, SB)
        return carry

    lax.fori_loop(0, RB // SB, first_body, 0)
    cp_xa(RB, S - RB, 4).wait()
    for k in range(2, 6):
        cp_wqkv(k).start()

    def qk_body(i, carry):
        @pl.when(i == 2)
        def _():
            cp_wqkv(1).wait()

        @pl.when(i == 4)
        def _():
            for k in range(2, 6):
                cp_wqkv(k).wait()

        for k in range(6):
            @pl.when(i == 2 + k)
            def _():
                start_wb(k)

        qk_block(i // nrb, pl.multiple_of((i % nrb) * RB, RB), RB)
        return carry

    lax.fori_loop(1, 4 * nrb, qk_body, 0)

    def v_body(i, carry):
        c = i // nrb
        r0 = (i % nrb) * RB

        @pl.when(i == 0)
        def _():
            for j in range(8):
                cp_wob(j).start()

        @pl.when(i == 1)
        def _():
            cp_xb.start()

        @pl.when(i == 2)
        def _():
            cp_woa.start()

        quarter = wb.at[pl.ds(4 * i, 4)]
        pltpu.make_async_copy(quarter, quarter, wsems.at[i]).wait()

        nsub = RB // SB
        npc = NPC // nsub
        nr = (D // 2) // (NPC // 12)
        for u in range(nsub):
            x = xa[pl.ds(pl.multiple_of(r0 + u * SB, SB), SB), :]
            y = _dot(x, wqkv[4 + c])
            yt = y.T.astype(BF16)
            for k in range(SB // KC):
                vt[(r0 + u * SB) // KC + k, pl.ds(pl.multiple_of(c * CB, CB), CB), :] = (
                    yt[:, k * KC:(k + 1) * KC])
            for n in range(npc):
                j, rest = divmod(u * npc + n, NPC // 4)
                m, part = divmod(rest, NPC // 12)
                rows = pl.ds(part * nr, nr)
                col = (n * 4 // npc) * 128
                row = ((n * 4 % npc) // 4) * (SB * 4 // npc) // 8 * 8
                sh = ((pltpu.bitcast(y[row:row + 8, col:col + 128], U32) >> 31) >> 1) + 16
                sh = jnp.tile(sh, (nr // 8, 1))
                a = quarter[j, m, 0, rows, :]
                b = quarter[j, m, 1, rows, :]
                quarter[j, m, 0, rows, :] = (a & 0xFFFF) | (b << sh)
                quarter[j, m, 1, rows, :] = (a >> sh) | (b & jnp.uint32(0xFFFF0000))
        return carry

    lax.fori_loop(0, 2 * nrb, v_body, 0)

    lane_grp = lax.broadcasted_iota(jnp.int32, (QB // 2, 128), 1) // DA
    qk32 = qk.bitcast(U32)
    vt32 = vt.bitcast(U32)

    def flush_tiles(g, k0, n):
        for k in range(n):
            o = ot[k0 + k, pl.ds(pl.multiple_of(g * 128, 128), 128), :]
            on[g, pl.ds(pl.multiple_of((k0 + k) * 128, 128), 128), :] = o.T.astype(BF16)

    def block_parts(na, w, nb, r, z):
        st = dict(m=None, l=None, acc=None)

        def qk_part(c):
            h = na // NQ
            if c == 0:
                qt = qk32[h // 4, pl.ds(pl.multiple_of((na % NQ) * (QB // 2), QB // 2), QB // 2), :]
                st['q'] = pltpu.bitcast(
                    jnp.where(lane_grp == h % 4, qt, jnp.zeros_like(qt)), BF16)
            kc = pltpu.bitcast(qk32[8 + h // 4, pl.ds(c * (KC // 2), KC // 2), :], BF16)
            s = _dot(kc, st['q'], NT)
            sbuf[w][pl.ds(c * KC, KC), :] = s
            mc = jnp.max(s.reshape(KC // 8, 8, QB), axis=0)
            st['m'] = mc if st['m'] is None else jnp.maximum(st['m'], mc)
            if c == NC - 1:
                mbuf[w][...] = st['m']

        def pv_part(c):
            if c == 0:
                st['mb'] = jnp.broadcast_to(
                    jnp.max(mbuf[r][...], axis=0, keepdims=True), (8, QB))
            ps = [None] * (KC // 16)
            for i in reversed(range(KC // 16)):
                base = c * KC + i * 16
                p1 = jnp.exp2(sbuf[r][pl.ds(z + base + 8, 8), :] - st['mb'])
                p0 = jnp.exp2(sbuf[r][pl.ds(z + base, 8), :] - st['mb'])
                st['l'] = p0 if st['l'] is None else st['l'] + p0
                st['l'] = st['l'] + p1
                ps[i] = jnp.concatenate([p0, p1], axis=0).astype(BF16)
            h = nb // NQ
            v = pltpu.bitcast(
                vt32[c, pl.ds(pl.multiple_of(h * (DA // 2), DA // 2), DA // 2), :], BF16)
            d = _dot(v, jnp.concatenate(ps, axis=0))
            st['acc'] = d if st['acc'] is None else st['acc'] + d
            if c == NC - 1:
                o = st['acc'] / jnp.sum(st['l'], axis=0, keepdims=True)
                for t in range(QB // 128):
                    ot[(nb % NQ) * (QB // 128) + t, pl.ds(pl.multiple_of(h * DA, DA), DA), :] = (
                        o[:, t * 128:(t + 1) * 128])

        return ([(qk_part, c) for c in range(NC)] if na is not None else [],
                [(pv_part, c) for c in range(NC)] if nb is not None else [])

    for f, c in block_parts(0, 0, None, None, None)[0]:
        f(c)
    ot[:, pl.ds(0, 128), :] = jnp.zeros((S // 128, 128, 128), F32)

    cp_xb.wait()
    pltpu.make_async_copy(wob, wob, sems.at[13]).wait()

    hbuf[pl.ds(SEG, MEM), :] = mem_ref[...].astype(F32)
    row = lax.broadcasted_iota(jnp.int32, (LB, LB), 0)
    col = lax.broadcasted_iota(jnp.int32, (LB, LB), 1)
    mask = (row >= SEG) | (col >= SEG) | (col <= row)
    bscale = DB ** -0.5

    def step(s, last=False):
        rows = pl.ds(pl.multiple_of(s * SEG, SEG), SEG)
        hbuf[pl.ds(0, SEG), :] = xb[rows, :].astype(F32)
        z = pl.multiple_of(zero[0], 8)
        qk0, pv0 = block_parts(2 * s + 1, 1, 2 * s, 0, z)
        qk1, pv1 = block_parts(None if last else 2 * s + 2, 0, 2 * s + 1, 1, z)
        qk_parts, pv_parts = qk0 + qk1, pv0 + pv1
        flush_tiles(jnp.maximum(s // 8 - 1, 0), (s % 8) * 2, 2)
        gw = gw_ref[...].reshape(1, D).astype(F32)
        g = jax.nn.sigmoid(jnp.sum(xa[rows, :].astype(F32) * gw, axis=1, keepdims=True))
        gate[rows, :] = jnp.broadcast_to(g, (SEG, 128))

        def proj(h):
            w = jnp.concatenate(
                [pltpu.bitcast(wb[h // 2, i, h % 2], BF16) for i in range(3)], axis=1)
            y = _dot(hbuf[...], w)
            return _round(y[:, :DB]), y[:, DB:2 * DB].astype(BF16), y[:, 2 * DB:].astype(BF16)

        def scores(q, k):
            sc = jnp.where(mask, _dot(q, k, NT) * bscale, -1000000000.0)
            e = jnp.exp(sc - jnp.max(sc, axis=1, keepdims=True))
            return _round(e), jnp.sum(e, axis=1, keepdims=True)

        def attend(e, l, v):
            return _round(_dot(e, v) / l)

        def oproj(h, o):
            w = jnp.concatenate(
                [pltpu.bitcast(wob[j, pl.ds(h * (DB // 2), DB // 2), :], BF16)
                 for j in range(D // 128)], axis=1)
            return _dot(o[:SEG] if last else o, w)

        def att(parts, t):
            if 0 <= t < len(parts):
                f, c = parts[t]
                f(c)

        qkv, el, oo = {}, {}, {}
        acc = None
        for t in range(HB + 4):
            att(qk_parts, t - 4)
            att(pv_parts, t - 4)
            if t < HB:
                qkv[t] = proj(t)
            if 0 <= t - 1 < HB:
                el[t - 1] = scores(qkv[t - 1][0], qkv[t - 1][1])
            if 0 <= t - 3 < HB:
                oo[t - 3] = attend(*el[t - 3], qkv[t - 3][2])
            if 0 <= t - 4 < HB:
                y = oproj(t - 4, oo[t - 4])
                acc = y if acc is None else acc + y
        if not last:
            hbuf[pl.ds(SEG, MEM), :] = _round(acc[SEG:])
        bout[rows, :] = (1.0 - g) * acc[:SEG]

    def step_body(s, carry):
        step(s)
        return carry

    zero[0] = 0
    lax.fori_loop(0, NSEG - 1, step_body, 0)
    step(NSEG - 1, last=True)
    flush_tiles(HA // 4 - 1, 0, S // 128)

    cp_woa.wait()

    def out_body(i, carry):
        for u in range(RB // SB):
            rows = pl.ds(pl.multiple_of(i * RB + u * SB, SB), SB)
            o = jnp.concatenate([on[k, rows, :] for k in range(D // 128)], axis=1)
            a = _dot(o, woa[...])
            g = jnp.tile(gate[rows, :], (1, D // 128))
            outv[rows, :] = (g * a + bout[rows, :]).astype(BF16)
            pltpu.make_async_copy(outv.at[rows], out_hbm.at[rows], sems.at[14]).start()
        return carry

    lax.fori_loop(0, S // RB, out_body, 0)
    pltpu.make_async_copy(outv, out_hbm, sems.at[14]).wait()


@jax.jit
def pallas_gated_mix__softmax_full_mha__memory_aug_recurrent_mem_tr__prompt_kernel(
    A_x, A_wqkv, A_wo, B_x, B_mem0, B_Wq, B_Wk, B_Wv, B_Wo, B_seg_len, gate_w,
):
    del B_seg_len
    hbm = pl.BlockSpec(memory_space=pl.ANY)
    vmem = pl.BlockSpec(memory_space=pltpu.VMEM)
    split_d = (D // 2, 2, HB, DB)
    out = pl.pallas_call(
        _kernel,
        out_shape=jax.ShapeDtypeStruct((S, D), BF16),
        in_specs=[hbm, hbm, hbm, hbm, vmem, hbm, hbm, hbm, hbm, vmem],
        out_specs=hbm,
        scratch_shapes=[
            pltpu.VMEM((S, D), BF16),
            pltpu.VMEM((3 * D // CB, D, CB), BF16),
            pltpu.VMEM((D, D), BF16),
            pltpu.VMEM((S, D), BF16),
            pltpu.VMEM((HB // 2, 3, 2, D // 2, 128), U32),
            pltpu.VMEM((D // 128, HB * DB // 2, 128), U32),
            pltpu.VMEM((16, S, 128), BF16),
            pltpu.VMEM((NC, D, KC), BF16),
            pltpu.VMEM((S // 128, D, 128), F32),
            pltpu.VMEM((D // 128, S, 128), BF16),
            [pltpu.VMEM((S, QB), F32) for _ in range(2)],
            [pltpu.VMEM((8, QB), F32) for _ in range(2)],
            pltpu.VMEM((S, D), F32),
            pltpu.VMEM((S, 128), F32),
            pltpu.VMEM((LB, D), F32),
            pltpu.VMEM((S, D), BF16),
            pltpu.SMEM((1,), jnp.int32),
            pltpu.SemaphoreType.DMA((15,)),
            pltpu.SemaphoreType.DMA((4,)),
        ],
        compiler_params=pltpu.CompilerParams(vmem_limit_bytes=120 * 1024 * 1024),
        name="gated_mix",
    )(
        A_x.reshape(S, D), A_wqkv, A_wo, B_x.reshape(S, D), B_mem0.reshape(MEM, D),
        B_Wq.reshape(split_d), B_Wk.reshape(split_d), B_Wv.reshape(split_d),
        B_Wo.reshape(HB * DB, D), gate_w,
    )
    return out.reshape(1, S, D)
```

```python
import math

import jax
import jax.numpy as jnp
from jax import lax
import jax.experimental.pallas as pl
import jax.experimental.pallas.tpu as pltpu

F32 = jnp.float32
BF16 = jnp.bfloat16
U32 = jnp.uint32

S = 2048
D = 1024
HA = 32
DA = D // HA
HB = 32
DB = 128
MEM = 8
SEG = 32
LB = SEG + MEM
NSEG = S // SEG

QB = 512
KC = 128
NQ = S // QB
NC = S // KC
CB = 512
RB = 1024
SB = 256
NPC = 192

LOG2E = math.log2(math.e)
NN = (((1,), (0,)), ((), ()))
NT = (((1,), (1,)), ((), ()))


def _dot(a, b, dims=NN):
    return lax.dot_general(a, b, dims, preferred_element_type=F32)


def _round(x):
    return x.astype(BF16).astype(F32)


def _kernel(xa_hbm, wqkv_hbm, woa_hbm, mem_ref, wq_hbm, wk_hbm, wv_hbm,
            wob_hbm, gw_ref, out_hbm,
            xa, wqkv, woa, wb, wob, qk, vt, ot, on, sbuf, mbuf, bout, gate,
            hbuf, outv, zero, sems, wsems):
    def cp_xa(r0, n, sem):
        return pltpu.make_async_copy(
            xa_hbm.at[pl.ds(r0, n)], xa.at[pl.ds(r0, n)], sems.at[sem])

    def cp_wqkv(c):
        return pltpu.make_async_copy(
            wqkv_hbm.at[:, pl.ds(c * CB, CB)], wqkv.at[c], sems.at[5 + c])

    cp_woa = pltpu.make_async_copy(woa_hbm, woa, sems.at[11])

    def cp_wob(j):
        return pltpu.make_async_copy(
            wob_hbm.at[:, pl.ds(j * 128, 128)], wob.bitcast(BF16).at[j], sems.at[12])

    def start_wb(part):
        for n in range(16 * part, 16 * part + 16):
            j, i, c = n // 6, (n // 2) % 3, n % 2
            w32 = (wq_hbm, wk_hbm, wv_hbm)[i].bitcast(U32)
            pltpu.make_async_copy(
                w32.at[:, c, j, :], wb.at[j, i, c], wsems.at[j // 4]).start()

    cp_wqkv(0).start()
    cp_xa(0, SB, 0).start()

    qscale = (DA ** -0.5) * LOG2E
    nrb = S // RB

    def qk_block(c, r0, n):
        x = xa[pl.ds(r0, n), :]
        y = _dot(x, wqkv[c])
        y = (y * jnp.where(c < 2, qscale, 1.0).astype(F32)).astype(BF16)
        for g in range(CB // 128):
            qk[c * (CB // 128) + g, pl.ds(r0, n), :] = y[:, g * 128:(g + 1) * 128]

    cp_wqkv(0).wait()

    def first_body(i, carry):
        r0 = pl.multiple_of(i * SB, SB)
        cp_xa(r0, SB, i).wait()

        @pl.when(i == 0)
        def _():
            for k in range(1, RB // SB):
                cp_xa(k * SB, SB, k).start()

        @pl.when(i == 1)
        def _():
            cp_xa(RB, S - RB, 4).start()
            cp_wqkv(1).start()

        qk_block(0, r0, SB)
        return carry

    lax.fori_loop(0, RB // SB, first_body, 0)
    cp_xa(RB, S - RB, 4).wait()
    for k in range(2, 6):
        cp_wqkv(k).start()

    def qk_body(i, carry):
        @pl.when(i == 2)
        def _():
            cp_wqkv(1).wait()

        @pl.when(i == 4)
        def _():
            for k in range(2, 6):
                cp_wqkv(k).wait()

        for k in range(6):
            @pl.when(i == 2 + k)
            def _():
                start_wb(k)

        qk_block(i // nrb, pl.multiple_of((i % nrb) * RB, RB), RB)
        return carry

    lax.fori_loop(1, 4 * nrb, qk_body, 0)

    def v_body(i, carry):
        c = i // nrb
        r0 = (i % nrb) * RB

        @pl.when(i == 0)
        def _():
            for j in range(8):
                cp_wob(j).start()

        @pl.when(i == 1)
        def _():
            cp_woa.start()

        quarter = wb.at[pl.ds(4 * i, 4)]
        pltpu.make_async_copy(quarter, quarter, wsems.at[i]).wait()

        nsub = RB // SB
        npc = NPC // nsub
        nr = (D // 2) // (NPC // 12)
        for u in range(nsub):
            x = xa[pl.ds(pl.multiple_of(r0 + u * SB, SB), SB), :]
            y = _dot(x, wqkv[4 + c])
            yt = y.T.astype(BF16)
            for k in range(SB // KC):
                vt[(r0 + u * SB) // KC + k, pl.ds(pl.multiple_of(c * CB, CB), CB), :] = (
                    yt[:, k * KC:(k + 1) * KC])
            for n in range(npc):
                j, rest = divmod(u * npc + n, NPC // 4)
                m, part = divmod(rest, NPC // 12)
                rows = pl.ds(part * nr, nr)
                col = (n * 4 // npc) * 128
                row = ((n * 4 % npc) // 4) * (SB * 4 // npc) // 8 * 8
                sh = ((pltpu.bitcast(y[row:row + 8, col:col + 128], U32) >> 31) >> 1) + 16
                sh = jnp.tile(sh, (nr // 8, 1))
                a = quarter[j, m, 0, rows, :]
                b = quarter[j, m, 1, rows, :]
                quarter[j, m, 0, rows, :] = (a & 0xFFFF) | (b << sh)
                quarter[j, m, 1, rows, :] = (a >> sh) | (b & jnp.uint32(0xFFFF0000))
        return carry

    lax.fori_loop(0, 2 * nrb, v_body, 0)

    lane_grp = lax.broadcasted_iota(jnp.int32, (QB // 2, 128), 1) // DA
    qk32 = qk.bitcast(U32)
    vt32 = vt.bitcast(U32)

    def flush_tiles(g, k0, n):
        for k in range(n):
            o = ot[k0 + k, pl.ds(pl.multiple_of(g * 128, 128), 128), :]
            on[g, pl.ds(pl.multiple_of((k0 + k) * 128, 128), 128), :] = o.T.astype(BF16)

    def block_parts(na, w, nb, r, z):
        st = dict(m=None, l=None, acc=None)

        def qk_part(c):
            h = na // NQ
            if c == 0:
                qt = qk32[h // 4, pl.ds(pl.multiple_of((na % NQ) * (QB // 2), QB // 2), QB // 2), :]
                st['q'] = pltpu.bitcast(
                    jnp.where(lane_grp == h % 4, qt, jnp.zeros_like(qt)), BF16)
            kc = pltpu.bitcast(qk32[8 + h // 4, pl.ds(c * (KC // 2), KC // 2), :], BF16)
            s = _dot(kc, st['q'], NT)
            sbuf[w][pl.ds(c * KC, KC), :] = s
            mc = jnp.max(s.reshape(KC // 8, 8, QB), axis=0)
            st['m'] = mc if st['m'] is None else jnp.maximum(st['m'], mc)
            if c == NC - 1:
                mbuf[w][...] = st['m']

        def pv_part(c):
            if c == 0:
                st['mb'] = jnp.broadcast_to(
                    jnp.max(mbuf[r][...], axis=0, keepdims=True), (8, QB))
            ps = [None] * (KC // 16)
            for i in reversed(range(KC // 16)):
                base = c * KC + i * 16
                p1 = jnp.exp2(sbuf[r][pl.ds(z + base + 8, 8), :] - st['mb'])
                p0 = jnp.exp2(sbuf[r][pl.ds(z + base, 8), :] - st['mb'])
                st['l'] = p0 if st['l'] is None else st['l'] + p0
                st['l'] = st['l'] + p1
                ps[i] = jnp.concatenate([p0, p1], axis=0).astype(BF16)
            h = nb // NQ
            v = pltpu.bitcast(
                vt32[c, pl.ds(pl.multiple_of(h * (DA // 2), DA // 2), DA // 2), :], BF16)
            d = _dot(v, jnp.concatenate(ps, axis=0))
            st['acc'] = d if st['acc'] is None else st['acc'] + d
            if c == NC - 1:
                o = st['acc'] / jnp.sum(st['l'], axis=0, keepdims=True)
                for t in range(QB // 128):
                    ot[(nb % NQ) * (QB // 128) + t, pl.ds(pl.multiple_of(h * DA, DA), DA), :] = (
                        o[:, t * 128:(t + 1) * 128])

        return ([(qk_part, c) for c in range(NC)] if na is not None else [],
                [(pv_part, c) for c in range(NC)] if nb is not None else [])

    for f, c in block_parts(0, 0, None, None, None)[0]:
        f(c)
    ot[:, pl.ds(0, 128), :] = jnp.zeros((S // 128, 128, 128), F32)

    pltpu.make_async_copy(wob, wob, sems.at[12]).wait()

    hbuf[pl.ds(SEG, MEM), :] = mem_ref[...].astype(F32)
    row = lax.broadcasted_iota(jnp.int32, (LB, LB), 0)
    col = lax.broadcasted_iota(jnp.int32, (LB, LB), 1)
    mask = (row >= SEG) | (col >= SEG) | (col <= row)
    bscale = DB ** -0.5

    def step(s, last=False):
        rows = pl.ds(pl.multiple_of(s * SEG, SEG), SEG)
        xs = xa[rows, :].astype(F32)
        hbuf[pl.ds(0, SEG), :] = xs
        z = pl.multiple_of(zero[0], 8)
        qk0, pv0 = block_parts(2 * s + 1, 1, 2 * s, 0, z)
        qk1, pv1 = block_parts(None if last else 2 * s + 2, 0, 2 * s + 1, 1, z)
        qk_parts, pv_parts = qk0 + qk1, pv0 + pv1
        flush_tiles(jnp.maximum(s // 8 - 1, 0), (s % 8) * 2, 2)
        gw = gw_ref[...].reshape(1, D).astype(F32)
        g = jax.nn.sigmoid(jnp.sum(xs * gw, axis=1, keepdims=True))
        gate[rows, :] = jnp.broadcast_to(g, (SEG, 128))

        def proj(h):
            w = jnp.concatenate(
                [pltpu.bitcast(wb[h // 2, i, h % 2], BF16) for i in range(3)], axis=1)
            y = _dot(hbuf[...], w)
            return _round(y[:, :DB]), y[:, DB:2 * DB].astype(BF16), y[:, 2 * DB:].astype(BF16)

        def scores(q, k):
            sc = jnp.where(mask, _dot(q, k, NT) * bscale, -1000000000.0)
            e = jnp.exp(sc - jnp.max(sc, axis=1, keepdims=True))
            return _round(e), jnp.sum(e, axis=1, keepdims=True)

        def attend(e, l, v):
            return _round(_dot(e, v) / l)

        def oproj(h, o):
            w = jnp.concatenate(
                [pltpu.bitcast(wob[j, pl.ds(h * (DB // 2), DB // 2), :], BF16)
                 for j in range(D // 128)], axis=1)
            return _dot(o[:SEG] if last else o, w)

        def att(parts, t):
            if 0 <= t < len(parts):
                f, c = parts[t]
                f(c)

        qkv, el, oo = {}, {}, {}
        acc = None
        for t in range(HB + 4):
            att(qk_parts, t - 4)
            att(pv_parts, t - 4)
            if t < HB:
                qkv[t] = proj(t)
            if 0 <= t - 1 < HB:
                el[t - 1] = scores(qkv[t - 1][0], qkv[t - 1][1])
            if 0 <= t - 3 < HB:
                oo[t - 3] = attend(*el[t - 3], qkv[t - 3][2])
            if 0 <= t - 4 < HB:
                y = oproj(t - 4, oo[t - 4])
                acc = y if acc is None else acc + y
        if not last:
            hbuf[pl.ds(SEG, MEM), :] = _round(acc[SEG:])
        bout[rows, :] = (1.0 - g) * acc[:SEG]

    def step_body(s, carry):
        step(s)
        return carry

    zero[0] = 0
    lax.fori_loop(0, NSEG - 1, step_body, 0)
    step(NSEG - 1, last=True)
    flush_tiles(HA // 4 - 1, 0, S // 128)

    cp_woa.wait()

    def out_body(i, carry):
        for u in range(RB // SB):
            rows = pl.ds(pl.multiple_of(i * RB + u * SB, SB), SB)
            o = jnp.concatenate([on[k, rows, :] for k in range(D // 128)], axis=1)
            a = _dot(o, woa[...])
            g = jnp.tile(gate[rows, :], (1, D // 128))
            outv[rows, :] = (g * a + bout[rows, :]).astype(BF16)
            pltpu.make_async_copy(outv.at[rows], out_hbm.at[rows], sems.at[13]).start()
        return carry

    lax.fori_loop(0, S // RB, out_body, 0)
    pltpu.make_async_copy(outv, out_hbm, sems.at[13]).wait()


@jax.jit
def pallas_gated_mix__softmax_full_mha__memory_aug_recurrent_mem_tr__prompt_kernel(
    A_x, A_wqkv, A_wo, B_x, B_mem0, B_Wq, B_Wk, B_Wv, B_Wo, B_seg_len, gate_w,
):
    del B_x
    del B_seg_len
    hbm = pl.BlockSpec(memory_space=pl.ANY)
    vmem = pl.BlockSpec(memory_space=pltpu.VMEM)
    split_d = (D // 2, 2, HB, DB)
    out = pl.pallas_call(
        _kernel,
        out_shape=jax.ShapeDtypeStruct((S, D), BF16),
        in_specs=[hbm, hbm, hbm, vmem, hbm, hbm, hbm, hbm, vmem],
        out_specs=hbm,
        scratch_shapes=[
            pltpu.VMEM((S, D), BF16),
            pltpu.VMEM((3 * D // CB, D, CB), BF16),
            pltpu.VMEM((D, D), BF16),
            pltpu.VMEM((HB // 2, 3, 2, D // 2, 128), U32),
            pltpu.VMEM((D // 128, HB * DB // 2, 128), U32),
            pltpu.VMEM((16, S, 128), BF16),
            pltpu.VMEM((NC, D, KC), BF16),
            pltpu.VMEM((S // 128, D, 128), F32),
            pltpu.VMEM((D // 128, S, 128), BF16),
            [pltpu.VMEM((S, QB), F32) for _ in range(2)],
            [pltpu.VMEM((8, QB), F32) for _ in range(2)],
            pltpu.VMEM((S, D), F32),
            pltpu.VMEM((S, 128), F32),
            pltpu.VMEM((LB, D), F32),
            pltpu.VMEM((S, D), BF16),
            pltpu.SMEM((1,), jnp.int32),
            pltpu.SemaphoreType.DMA((14,)),
            pltpu.SemaphoreType.DMA((4,)),
        ],
        compiler_params=pltpu.CompilerParams(vmem_limit_bytes=120 * 1024 * 1024),
        name="gated_mix",
    )(
        A_x.reshape(S, D), A_wqkv, A_wo, B_mem0.reshape(MEM, D),
        B_Wq.reshape(split_d), B_Wk.reshape(split_d), B_Wv.reshape(split_d),
        B_Wo.reshape(HB * DB, D), gate_w,
    )
    return out.reshape(1, S, D)
```

```python
import math

import jax
import jax.numpy as jnp
from jax import lax
import jax.experimental.pallas as pl
import jax.experimental.pallas.tpu as pltpu

F32 = jnp.float32
BF16 = jnp.bfloat16
U32 = jnp.uint32

S = 2048
D = 1024
HA = 32
DA = D // HA
HB = 32
DB = 128
MEM = 8
SEG = 32
LB = SEG + MEM
NSEG = S // SEG

QB = 512
KC = 128
NQ = S // QB
NC = S // KC
CB = 512
RB = 1024
SB = 256
NPC = 192

LOG2E = math.log2(math.e)
NN = (((1,), (0,)), ((), ()))
NT = (((1,), (1,)), ((), ()))


def _dot(a, b, dims=NN):
    return lax.dot_general(a, b, dims, preferred_element_type=F32)


def _round(x):
    return x.astype(BF16).astype(F32)


def _kernel(xa_hbm, wqkv_hbm, woa_hbm, mem_hbm, wq_hbm, wk_hbm, wv_hbm,
            wob_hbm, gw_hbm, out_hbm,
            xa, wqkv, woa, wb, wob, qk, vt, ot, on, sbuf, mbuf, bout, gate,
            hbuf, outv, mem0, gwv, zero, sems, wsems):
    def cp_xa(r0, n, sem):
        return pltpu.make_async_copy(
            xa_hbm.at[pl.ds(r0, n)], xa.at[pl.ds(r0, n)], sems.at[sem])

    def cp_wqkv(c):
        return pltpu.make_async_copy(
            wqkv_hbm.at[:, pl.ds(c * CB, CB)], wqkv.at[c], sems.at[5 + c])

    cp_mem = pltpu.make_async_copy(mem_hbm, mem0, sems.at[14])
    cp_gw = pltpu.make_async_copy(gw_hbm, gwv, sems.at[15])
    cp_woa = pltpu.make_async_copy(woa_hbm, woa, sems.at[11])

    def cp_wob(j):
        return pltpu.make_async_copy(
            wob_hbm.at[:, pl.ds(j * 128, 128)], wob.bitcast(BF16).at[j], sems.at[12])

    def start_wb(part):
        for n in range(16 * part, 16 * part + 16):
            j, i, c = n // 6, (n // 2) % 3, n % 2
            w32 = (wq_hbm, wk_hbm, wv_hbm)[i].bitcast(U32)
            pltpu.make_async_copy(
                w32.at[:, c, j, :], wb.at[j, i, c], wsems.at[j // 4]).start()

    cp_wqkv(0).start()
    cp_xa(0, SB, 0).start()

    qscale = (DA ** -0.5) * LOG2E
    nrb = S // RB

    def qk_block(c, r0, n):
        x = xa[pl.ds(r0, n), :]
        y = _dot(x, wqkv[c])
        y = (y * jnp.where(c < 2, qscale, 1.0).astype(F32)).astype(BF16)
        for g in range(CB // 128):
            qk[c * (CB // 128) + g, pl.ds(r0, n), :] = y[:, g * 128:(g + 1) * 128]

    cp_wqkv(0).wait()

    def first_body(i, carry):
        r0 = pl.multiple_of(i * SB, SB)
        cp_xa(r0, SB, i).wait()

        @pl.when(i == 0)
        def _():
            for k in range(1, RB // SB):
                cp_xa(k * SB, SB, k).start()

        @pl.when(i == 1)
        def _():
            cp_xa(RB, S - RB, 4).start()
            cp_wqkv(1).start()

        qk_block(0, r0, SB)
        return carry

    lax.fori_loop(0, RB // SB, first_body, 0)
    cp_xa(RB, S - RB, 4).wait()
    for k in range(2, 6):
        cp_wqkv(k).start()

    qk_block(0, RB, RB)

    def qk_body(i, carry):
        c = i + 1

        @pl.when(i == 0)
        def _():
            cp_wqkv(1).wait()

        @pl.when(i == 1)
        def _():
            for k in range(2, 6):
                cp_wqkv(k).wait()

        for k in range(3):
            @pl.when(i == k)
            def _():
                start_wb(2 * k)
                start_wb(2 * k + 1)

        for r in range(nrb):
            qk_block(c, r * RB, RB)
        return carry

    lax.fori_loop(0, 3, qk_body, 0)

    def v_block(i):
        c, r0 = i // nrb, (i % nrb) * RB
        quarter = wb.at[pl.ds(4 * i, 4)]
        nsub = RB // SB
        npc = NPC // nsub
        nr = (D // 2) // (NPC // 12)
        for u in range(nsub):
            y = _dot(xa[pl.ds(r0 + u * SB, SB), :], wqkv[4 + c])
            yt = y.T.astype(BF16)
            for k in range(SB // KC):
                vt[(r0 + u * SB) // KC + k, pl.ds(c * CB, CB), :] = yt[:, k * KC:(k + 1) * KC]
            for n in range(npc):
                j, rest = divmod(u * npc + n, NPC // 4)
                m, part = divmod(rest, NPC // 12)
                rows = pl.ds(part * nr, nr)
                col = (n * 4 // npc) * 128
                row = ((n * 4 % npc) // 4) * (SB * 4 // npc) // 8 * 8
                sh = ((pltpu.bitcast(y[row:row + 8, col:col + 128], U32) >> 31) >> 1) + 16
                sh = jnp.tile(sh, (nr // 8, 1))
                a = quarter[j, m, 0, rows, :]
                b = quarter[j, m, 1, rows, :]
                quarter[j, m, 0, rows, :] = (a & 0xFFFF) | (b << sh)
                quarter[j, m, 1, rows, :] = (a >> sh) | (b & jnp.uint32(0xFFFF0000))

    for j in range(8):
        cp_wob(j).start()
    cp_woa.start()
    cp_mem.start()
    cp_gw.start()
    for half in range(2):
        for i in range(2 * half, 2 * half + 2):
            quarter = wb.at[pl.ds(4 * i, 4)]
            pltpu.make_async_copy(quarter, quarter, wsems.at[i]).wait()
        for i in range(2 * half, 2 * half + 2):
            v_block(i)

    lane_grp = lax.broadcasted_iota(jnp.int32, (QB // 2, 128), 1) // DA
    qk32 = qk.bitcast(U32)
    vt32 = vt.bitcast(U32)

    def flush_tiles(g, k0, n):
        for k in range(n):
            o = ot[k0 + k, pl.ds(pl.multiple_of(g * 128, 128), 128), :]
            on[g, pl.ds(pl.multiple_of((k0 + k) * 128, 128), 128), :] = o.T.astype(BF16)

    def block_parts(na, w, nb, r, z):
        st = dict(m=None, l=None, acc=None)

        def qk_part(c):
            h = na // NQ
            if c == 0:
                qt = qk32[h // 4, pl.ds(pl.multiple_of((na % NQ) * (QB // 2), QB // 2), QB // 2), :]
                st['q'] = pltpu.bitcast(
                    jnp.where(lane_grp == h % 4, qt, jnp.zeros_like(qt)), BF16)
            kc = pltpu.bitcast(qk32[8 + h // 4, pl.ds(c * (KC // 2), KC // 2), :], BF16)
            s = _dot(kc, st['q'], NT)
            sbuf[w][pl.ds(c * KC, KC), :] = s
            mc = jnp.max(s.reshape(KC // 8, 8, QB), axis=0)
            st['m'] = mc if st['m'] is None else jnp.maximum(st['m'], mc)
            if c == NC - 1:
                mbuf[w][...] = st['m']

        def pv_part(c):
            if c == 0:
                st['mb'] = jnp.broadcast_to(
                    jnp.max(mbuf[r][...], axis=0, keepdims=True), (8, QB))
            ps = [None] * (KC // 16)
            for i in reversed(range(KC // 16)):
                base = c * KC + i * 16
                p1 = jnp.exp2(sbuf[r][pl.ds(z + base + 8, 8), :] - st['mb'])
                p0 = jnp.exp2(sbuf[r][pl.ds(z + base, 8), :] - st['mb'])
                st['l'] = p0 if st['l'] is None else st['l'] + p0
                st['l'] = st['l'] + p1
                ps[i] = jnp.concatenate([p0, p1], axis=0).astype(BF16)
            h = nb // NQ
            v = pltpu.bitcast(
                vt32[c, pl.ds(pl.multiple_of(h * (DA // 2), DA // 2), DA // 2), :], BF16)
            d = _dot(v, jnp.concatenate(ps, axis=0))
            st['acc'] = d if st['acc'] is None else st['acc'] + d
            if c == NC - 1:
                o = st['acc'] / jnp.sum(st['l'], axis=0, keepdims=True)
                for t in range(QB // 128):
                    ot[(nb % NQ) * (QB // 128) + t, pl.ds(pl.multiple_of(h * DA, DA), DA), :] = (
                        o[:, t * 128:(t + 1) * 128])

        return ([(qk_part, c) for c in range(NC)] if na is not None else [],
                [(pv_part, c) for c in range(NC)] if nb is not None else [])

    for f, c in block_parts(0, 0, None, None, None)[0]:
        f(c)
    ot[:, pl.ds(0, 128), :] = jnp.zeros((S // 128, 128, 128), F32)

    pltpu.make_async_copy(wob, wob, sems.at[12]).wait()
    cp_mem.wait()
    cp_gw.wait()

    hbuf[pl.ds(SEG, MEM), :] = mem0[...].astype(F32)
    row = lax.broadcasted_iota(jnp.int32, (LB, LB), 0)
    col = lax.broadcasted_iota(jnp.int32, (LB, LB), 1)
    mask = (row >= SEG) | (col >= SEG) | (col <= row)
    bscale = DB ** -0.5

    def step(s, last=False):
        rows = pl.ds(pl.multiple_of(s * SEG, SEG), SEG)
        xs = xa[rows, :].astype(F32)
        hbuf[pl.ds(0, SEG), :] = xs
        z = pl.multiple_of(zero[0], 8)
        qk0, pv0 = block_parts(2 * s + 1, 1, 2 * s, 0, z)
        qk1, pv1 = block_parts(None if last else 2 * s + 2, 0, 2 * s + 1, 1, z)
        qk_parts, pv_parts = qk0 + qk1, pv0 + pv1
        flush_tiles(jnp.maximum(s // 8 - 1, 0), (s % 8) * 2, 2)
        gw = gwv[...].reshape(1, D).astype(F32)
        g = jax.nn.sigmoid(jnp.sum(xs * gw, axis=1, keepdims=True))
        gate[rows, :] = jnp.broadcast_to(g, (SEG, 128))

        def proj(h):
            w = jnp.concatenate(
                [pltpu.bitcast(wb[h // 2, i, h % 2], BF16) for i in range(3)], axis=1)
            y = _dot(hbuf[...], w)
            return _round(y[:, :DB]), y[:, DB:2 * DB].astype(BF16), y[:, 2 * DB:].astype(BF16)

        def scores(q, k):
            sc = jnp.where(mask, _dot(q, k, NT) * bscale, -1000000000.0)
            e = jnp.exp(sc - jnp.max(sc, axis=1, keepdims=True))
            return _round(e), jnp.sum(e, axis=1, keepdims=True)

        def attend(e, l, v):
            return _round(_dot(e, v) / l)

        def oproj(h, o):
            w = jnp.concatenate(
                [pltpu.bitcast(wob[j, pl.ds(h * (DB // 2), DB // 2), :], BF16)
                 for j in range(D // 128)], axis=1)
            return _dot(o[:SEG] if last else o, w)

        def att(parts, t):
            if 0 <= t < len(parts):
                f, c = parts[t]
                f(c)

        qkv, el, oo = {}, {}, {}
        acc = None
        for t in range(HB + 4):
            att(qk_parts, t - 4)
            att(pv_parts, t - 4)
            if t < HB:
                qkv[t] = proj(t)
            if 0 <= t - 1 < HB:
                el[t - 1] = scores(qkv[t - 1][0], qkv[t - 1][1])
            if 0 <= t - 3 < HB:
                oo[t - 3] = attend(*el[t - 3], qkv[t - 3][2])
            if 0 <= t - 4 < HB:
                y = oproj(t - 4, oo[t - 4])
                acc = y if acc is None else acc + y
        if not last:
            hbuf[pl.ds(SEG, MEM), :] = _round(acc[SEG:])
        bout[rows, :] = (1.0 - g) * acc[:SEG]

    def step_body(s, carry):
        step(s)
        return carry

    zero[0] = 0
    lax.fori_loop(0, NSEG - 1, step_body, 0)
    step(NSEG - 1, last=True)
    flush_tiles(HA // 4 - 1, 0, S // 128)

    cp_woa.wait()

    r0 = 0
    for n in (512, 512, 512, 256, 128, 64, 64):
        rows = pl.ds(r0, n)
        o = jnp.concatenate([on[k, rows, :] for k in range(D // 128)], axis=1)
        a = _dot(o, woa[...])
        g = jnp.tile(gate[rows, :], (1, D // 128))
        outv[rows, :] = (g * a + bout[rows, :]).astype(BF16)
        pltpu.make_async_copy(outv.at[rows], out_hbm.at[rows], sems.at[13]).start()
        r0 += n
    assert r0 == S
    pltpu.make_async_copy(outv, out_hbm, sems.at[13]).wait()


@jax.jit
def pallas_gated_mix__softmax_full_mha__memory_aug_recurrent_mem_tr__prompt_kernel(
    A_x, A_wqkv, A_wo, B_x, B_mem0, B_Wq, B_Wk, B_Wv, B_Wo, B_seg_len, gate_w,
):
    del B_x
    del B_seg_len
    hbm = pl.BlockSpec(memory_space=pl.ANY)
    split_d = (D // 2, 2, HB, DB)
    out = pl.pallas_call(
        _kernel,
        out_shape=jax.ShapeDtypeStruct((S, D), BF16),
        in_specs=[hbm] * 9,
        out_specs=hbm,
        scratch_shapes=[
            pltpu.VMEM((S, D), BF16),
            pltpu.VMEM((3 * D // CB, D, CB), BF16),
            pltpu.VMEM((D, D), BF16),
            pltpu.VMEM((HB // 2, 3, 2, D // 2, 128), U32),
            pltpu.VMEM((D // 128, HB * DB // 2, 128), U32),
            pltpu.VMEM((16, S, 128), BF16),
            pltpu.VMEM((NC, D, KC), BF16),
            pltpu.VMEM((S // 128, D, 128), F32),
            pltpu.VMEM((D // 128, S, 128), BF16),
            [pltpu.VMEM((S, QB), F32) for _ in range(2)],
            [pltpu.VMEM((8, QB), F32) for _ in range(2)],
            pltpu.VMEM((S, D), F32),
            pltpu.VMEM((S, 128), F32),
            pltpu.VMEM((LB, D), F32),
            pltpu.VMEM((S, D), BF16),
            pltpu.VMEM((MEM, D), BF16),
            pltpu.VMEM((D,), BF16),
            pltpu.SMEM((1,), jnp.int32),
            pltpu.SemaphoreType.DMA((16,)),
            pltpu.SemaphoreType.DMA((4,)),
        ],
        compiler_params=pltpu.CompilerParams(vmem_limit_bytes=120 * 1024 * 1024),
        name="gated_mix",
    )(
        A_x.reshape(S, D), A_wqkv, A_wo, B_mem0.reshape(MEM, D),
        B_Wq.reshape(split_d), B_Wk.reshape(split_d), B_Wv.reshape(split_d),
        B_Wo.reshape(HB * DB, D), gate_w,
    )
    return out.reshape(1, S, D)
```

```python
import math

import jax
import jax.numpy as jnp
from jax import lax
import jax.experimental.pallas as pl
import jax.experimental.pallas.tpu as pltpu

F32 = jnp.float32
BF16 = jnp.bfloat16
U32 = jnp.uint32

S = 2048
D = 1024
HA = 32
DA = D // HA
HB = 32
DB = 128
MEM = 8
SEG = 32
LB = SEG + MEM
NSEG = S // SEG

QB = 512
KC = 128
NQ = S // QB
NC = S // KC
CB = 512
RB = 1024
SB = 256
NPC = 192
ATT_SLOTS = [t for t in range(2 * NC + 2) if t not in (0, NC + 4)]

LOG2E = math.log2(math.e)
NN = (((1,), (0,)), ((), ()))
NT = (((1,), (1,)), ((), ()))


def _dot(a, b, dims=NN):
    return lax.dot_general(a, b, dims, preferred_element_type=F32)


def _round(x):
    return x.astype(BF16).astype(F32)


def _kernel(xa_hbm, wqkv_hbm, woa_hbm, mem_hbm, wq_hbm, wk_hbm, wv_hbm,
            wob_hbm, gw_hbm, out_hbm,
            xa, wqkv, woa, wb, wob, qk, vt, ot, on, sbuf, mbuf, bout, gate,
            hbuf, outv, mem0, gwv, zero, sems, wsems):
    def cp_xa(r0, n, sem):
        return pltpu.make_async_copy(
            xa_hbm.at[pl.ds(r0, n)], xa.at[pl.ds(r0, n)], sems.at[sem])

    def cp_wqkv(c):
        return pltpu.make_async_copy(
            wqkv_hbm.at[:, pl.ds(c * CB, CB)], wqkv.at[c], sems.at[5 + c])

    cp_mem = pltpu.make_async_copy(mem_hbm, mem0, sems.at[14])
    cp_gw = pltpu.make_async_copy(gw_hbm, gwv, sems.at[15])
    cp_woa = pltpu.make_async_copy(woa_hbm, woa, sems.at[11])

    def cp_wob(j):
        return pltpu.make_async_copy(
            wob_hbm.at[:, pl.ds(j * 128, 128)], wob.bitcast(BF16).at[j], sems.at[12])

    def start_wb(part):
        for n in range(16 * part, 16 * part + 16):
            j, i, c = n // 6, (n // 2) % 3, n % 2
            w32 = (wq_hbm, wk_hbm, wv_hbm)[i].bitcast(U32)
            pltpu.make_async_copy(
                w32.at[:, c, j, :], wb.at[j, i, c], wsems.at[j // 4]).start()

    cp_wqkv(0).start()
    cp_xa(0, SB, 0).start()

    qscale = (DA ** -0.5) * LOG2E
    nrb = S // RB

    def qk_block(c, r0, n):
        x = xa[pl.ds(r0, n), :]
        y = _dot(x, wqkv[c])
        y = (y * jnp.where(c < 2, qscale, 1.0).astype(F32)).astype(BF16)
        for g in range(CB // 128):
            qk[c * (CB // 128) + g, pl.ds(r0, n), :] = y[:, g * 128:(g + 1) * 128]

    cp_wqkv(0).wait()

    def first_body(i, carry):
        r0 = pl.multiple_of(i * SB, SB)
        cp_xa(r0, SB, i).wait()

        @pl.when(i == 0)
        def _():
            for k in range(1, RB // SB):
                cp_xa(k * SB, SB, k).start()

        @pl.when(i == 1)
        def _():
            cp_xa(RB, S - RB, 4).start()
            cp_wqkv(1).start()

        qk_block(0, r0, SB)
        return carry

    lax.fori_loop(0, RB // SB, first_body, 0)
    cp_xa(RB, S - RB, 4).wait()
    for k in range(2, 6):
        cp_wqkv(k).start()

    qk_block(0, RB, RB)

    def qk_body(i, carry):
        c = i + 1

        @pl.when(i == 0)
        def _():
            cp_wqkv(1).wait()

        @pl.when(i == 1)
        def _():
            for k in range(2, 6):
                cp_wqkv(k).wait()

        for k in range(3):
            @pl.when(i == k)
            def _():
                start_wb(2 * k)
                start_wb(2 * k + 1)

        for r in range(nrb):
            qk_block(c, r * RB, RB)
        return carry

    lax.fori_loop(0, 3, qk_body, 0)

    def v_block(i):
        c, r0 = i // nrb, (i % nrb) * RB
        quarter = wb.at[pl.ds(4 * i, 4)]
        nsub = RB // SB
        npc = NPC // nsub
        nr = (D // 2) // (NPC // 12)
        for u in range(nsub):
            y = _dot(xa[pl.ds(r0 + u * SB, SB), :], wqkv[4 + c])
            yt = y.T.astype(BF16)
            for k in range(SB // KC):
                vt[(r0 + u * SB) // KC + k, pl.ds(c * CB, CB), :] = yt[:, k * KC:(k + 1) * KC]
            for n in range(npc):
                j, rest = divmod(u * npc + n, NPC // 4)
                m, part = divmod(rest, NPC // 12)
                rows = pl.ds(part * nr, nr)
                col = (n * 4 // npc) * 128
                row = ((n * 4 % npc) // 4) * (SB * 4 // npc) // 8 * 8
                sh = ((pltpu.bitcast(y[row:row + 8, col:col + 128], U32) >> 31) >> 1) + 16
                sh = jnp.tile(sh, (nr // 8, 1))
                a = quarter[j, m, 0, rows, :]
                b = quarter[j, m, 1, rows, :]
                quarter[j, m, 0, rows, :] = (a & 0xFFFF) | (b << sh)
                quarter[j, m, 1, rows, :] = (a >> sh) | (b & jnp.uint32(0xFFFF0000))

    for j in range(8):
        cp_wob(j).start()
    cp_woa.start()
    cp_mem.start()
    cp_gw.start()
    for half in range(2):
        for i in range(2 * half, 2 * half + 2):
            quarter = wb.at[pl.ds(4 * i, 4)]
            pltpu.make_async_copy(quarter, quarter, wsems.at[i]).wait()
        for i in range(2 * half, 2 * half + 2):
            v_block(i)

    lane_grp = lax.broadcasted_iota(jnp.int32, (QB // 2, 128), 1) // DA
    qk32 = qk.bitcast(U32)
    vt32 = vt.bitcast(U32)

    def flush_tiles(g, k0, n):
        for k in range(n):
            o = ot[k0 + k, pl.ds(pl.multiple_of(g * 128, 128), 128), :]
            on[g, pl.ds(pl.multiple_of((k0 + k) * 128, 128), 128), :] = o.T.astype(BF16)

    def block_parts(na, w, nb, r, z):
        st = dict(m=None, l=None, acc=None)

        def qk_part(c):
            h = na // NQ
            if c == 0:
                qt = qk32[h // 4, pl.ds(pl.multiple_of((na % NQ) * (QB // 2), QB // 2), QB // 2), :]
                st['q'] = pltpu.bitcast(
                    jnp.where(lane_grp == h % 4, qt, jnp.zeros_like(qt)), BF16)
            kc = pltpu.bitcast(qk32[8 + h // 4, pl.ds(c * (KC // 2), KC // 2), :], BF16)
            s = _dot(kc, st['q'], NT)
            sbuf[w][pl.ds(c * KC, KC), :] = s
            for i in range(0, KC, 16):
                x = jnp.maximum(s[i:i + 8], s[i + 8:i + 16])
                st['m'] = x if st['m'] is None else jnp.maximum(st['m'], x)
            if c == NC - 1:
                mbuf[w][...] = st['m']

        def pv_part(c):
            if c == 0:
                st['mb'] = jnp.broadcast_to(
                    jnp.max(mbuf[r][...], axis=0, keepdims=True), (8, QB))
            ps = [None] * (KC // 16)
            for i in reversed(range(KC // 16)):
                base = c * KC + i * 16
                p1 = jnp.exp2(sbuf[r][pl.ds(z + base + 8, 8), :] - st['mb'])
                p0 = jnp.exp2(sbuf[r][pl.ds(z + base, 8), :] - st['mb'])
                st['l'] = p1 if st['l'] is None else st['l'] + p1
                st['l'] = st['l'] + p0
                ps[i] = jnp.concatenate([p0, p1], axis=0).astype(BF16)
            h = nb // NQ
            v = pltpu.bitcast(
                vt32[c, pl.ds(pl.multiple_of(h * (DA // 2), DA // 2), DA // 2), :], BF16)
            d = _dot(v, jnp.concatenate(ps, axis=0))
            st['acc'] = d if st['acc'] is None else st['acc'] + d
            if c == NC - 1:
                o = st['acc'] / jnp.sum(st['l'], axis=0, keepdims=True)
                for t in range(QB // 128):
                    ot[(nb % NQ) * (QB // 128) + t, pl.ds(pl.multiple_of(h * DA, DA), DA), :] = (
                        o[:, t * 128:(t + 1) * 128])

        return ([(qk_part, c) for c in range(NC)] if na is not None else [],
                [(pv_part, c) for c in range(NC)] if nb is not None else [])

    for f, c in block_parts(0, 0, None, None, None)[0]:
        f(c)
    ot[:, pl.ds(0, 128), :] = jnp.zeros((S // 128, 128, 128), F32)

    pltpu.make_async_copy(wob, wob, sems.at[12]).wait()
    cp_mem.wait()
    cp_gw.wait()

    hbuf[pl.ds(SEG, MEM), :] = mem0[...].astype(F32)
    row = lax.broadcasted_iota(jnp.int32, (LB, LB), 0)
    col = lax.broadcasted_iota(jnp.int32, (LB, LB), 1)
    mask = (row >= SEG) | (col >= SEG) | (col <= row)
    bscale = DB ** -0.5

    def step(s, last=False):
        rows = pl.ds(pl.multiple_of(s * SEG, SEG), SEG)
        hbuf[pl.ds(0, SEG), :] = xa[rows, :].astype(F32)
        z = pl.multiple_of(zero[0], 8)
        qk0, pv0 = block_parts(2 * s + 1, 1, 2 * s, 0, z)
        qk1, pv1 = block_parts(None if last else 2 * s + 2, 0, 2 * s + 1, 1, z)
        qk_parts, pv_parts = qk0 + qk1, pv0 + pv1

        def proj(h):
            w = jnp.concatenate(
                [pltpu.bitcast(wb[h // 2, i, h % 2], BF16) for i in range(3)], axis=1)
            y = _dot(hbuf[...], w)
            return _round(y[:, :DB]), y[:, DB:2 * DB].astype(BF16), y[:, 2 * DB:].astype(BF16)

        def scores(q, k):
            sc = jnp.where(mask, _dot(q, k, NT) * bscale, -1000000000.0)
            e = jnp.exp(sc - jnp.max(sc, axis=1, keepdims=True))
            return _round(e), jnp.sum(e, axis=1, keepdims=True)

        def attend(e, l, v):
            return _round(_dot(e, v) / l)

        def oproj(h, o):
            w = jnp.concatenate(
                [pltpu.bitcast(wob[j, pl.ds(h * (DB // 2), DB // 2), :], BF16)
                 for j in range(D // 128)], axis=1)
            return _dot(o[:SEG] if last else o, w)

        qkv, el, oo = {}, {}, {}
        acc = None
        for t in range(HB + 5):
            if t == 30:
                flush_tiles(jnp.maximum(s // 8 - 1, 0), (s % 8) * 2, 2)
                gw = gwv[...].reshape(1, D).astype(F32)
                g = jax.nn.sigmoid(
                    jnp.sum(hbuf[pl.ds(0, SEG), :] * gw, axis=1, keepdims=True))
                gate[rows, :] = jnp.broadcast_to(g, (SEG, 128))
            if t in ATT_SLOTS:
                for parts in (qk_parts, pv_parts):
                    for f, c in parts[ATT_SLOTS.index(t):][:1]:
                        f(c)
            if t < HB:
                qkv[t] = proj(t)
            if 0 <= t - 1 < HB:
                el[t - 1] = scores(qkv[t - 1][0], qkv[t - 1][1])
            if 0 <= t - 3 < HB:
                oo[t - 3] = attend(*el[t - 3], qkv[t - 3][2])
            if 0 <= t - 5 < HB:
                y = oproj(t - 5, oo[t - 5])
                acc = y if acc is None else acc + y
        if not last:
            hbuf[pl.ds(SEG, MEM), :] = _round(acc[SEG:])
        bout[rows, :] = (1.0 - g) * acc[:SEG]

    def step_body(s, carry):
        step(s)
        return carry

    zero[0] = 0
    lax.fori_loop(0, NSEG - 1, step_body, 0)
    step(NSEG - 1, last=True)
    flush_tiles(HA // 4 - 1, 0, S // 128)

    cp_woa.wait()

    r0 = 0
    for n in (512, 512, 512, 256, 128, 64, 64):
        rows = pl.ds(r0, n)
        o = jnp.concatenate([on[k, rows, :] for k in range(D // 128)], axis=1)
        a = _dot(o, woa[...])
        g = jnp.tile(gate[rows, :], (1, D // 128))
        outv[rows, :] = (g * a + bout[rows, :]).astype(BF16)
        pltpu.make_async_copy(outv.at[rows], out_hbm.at[rows], sems.at[13]).start()
        r0 += n
    assert r0 == S
    pltpu.make_async_copy(outv, out_hbm, sems.at[13]).wait()


@jax.jit
def pallas_gated_mix__softmax_full_mha__memory_aug_recurrent_mem_tr__prompt_kernel(
    A_x, A_wqkv, A_wo, B_x, B_mem0, B_Wq, B_Wk, B_Wv, B_Wo, B_seg_len, gate_w,
):
    del B_x
    del B_seg_len
    hbm = pl.BlockSpec(memory_space=pl.ANY)
    split_d = (D // 2, 2, HB, DB)
    out = pl.pallas_call(
        _kernel,
        out_shape=jax.ShapeDtypeStruct((S, D), BF16),
        in_specs=[hbm] * 9,
        out_specs=hbm,
        scratch_shapes=[
            pltpu.VMEM((S, D), BF16),
            pltpu.VMEM((3 * D // CB, D, CB), BF16),
            pltpu.VMEM((D, D), BF16),
            pltpu.VMEM((HB // 2, 3, 2, D // 2, 128), U32),
            pltpu.VMEM((D // 128, HB * DB // 2, 128), U32),
            pltpu.VMEM((16, S, 128), BF16),
            pltpu.VMEM((NC, D, KC), BF16),
            pltpu.VMEM((S // 128, D, 128), F32),
            pltpu.VMEM((D // 128, S, 128), BF16),
            [pltpu.VMEM((S, QB), F32) for _ in range(2)],
            [pltpu.VMEM((8, QB), F32) for _ in range(2)],
            pltpu.VMEM((S, D), F32),
            pltpu.VMEM((S, 128), F32),
            pltpu.VMEM((LB, D), F32),
            pltpu.VMEM((S, D), BF16),
            pltpu.VMEM((MEM, D), BF16),
            pltpu.VMEM((D,), BF16),
            pltpu.SMEM((1,), jnp.int32),
            pltpu.SemaphoreType.DMA((16,)),
            pltpu.SemaphoreType.DMA((4,)),
        ],
        compiler_params=pltpu.CompilerParams(vmem_limit_bytes=120 * 1024 * 1024),
        name="gated_mix",
    )(
        A_x.reshape(S, D), A_wqkv, A_wo, B_mem0.reshape(MEM, D),
        B_Wq.reshape(split_d), B_Wk.reshape(split_d), B_Wv.reshape(split_d),
        B_Wo.reshape(HB * DB, D), gate_w,
    )
    return out.reshape(1, S, D)
```

```python
import math

import jax
import jax.numpy as jnp
from jax import lax
import jax.experimental.pallas as pl
import jax.experimental.pallas.tpu as pltpu

F32 = jnp.float32
BF16 = jnp.bfloat16
U32 = jnp.uint32

S = 2048
D = 1024
HA = 32
DA = D // HA
HB = 32
DB = 128
MEM = 8
SEG = 32
LB = SEG + MEM
NSEG = S // SEG

QB = 512
KC = 128
NQ = S // QB
NC = S // KC
CB = 512
RB = 1024
SB = 256
NPC = 192
ATT_SLOTS = [t for t in range(2 * NC + 2) if t not in (0, NC + 4)]

LOG2E = math.log2(math.e)
NN = (((1,), (0,)), ((), ()))
NT = (((1,), (1,)), ((), ()))


def _dot(a, b, dims=NN):
    return lax.dot_general(a, b, dims, preferred_element_type=F32)


def _round(x):
    return x.astype(BF16).astype(F32)


def _kernel(xa_hbm, wqkv_hbm, woa_hbm, mem_hbm, wq_hbm, wk_hbm, wv_hbm,
            wob_hbm, gw_hbm, out_hbm,
            xa, wqkv, woa, wb, wob, qk, vt, ot, on, sbuf, mbuf, bout, gate,
            hbuf, outv, mem0, gwv, zero, sems, wsems):
    def cp_xa(r0, n, sem):
        return pltpu.make_async_copy(
            xa_hbm.at[pl.ds(r0, n)], xa.at[pl.ds(r0, n)], sems.at[sem])

    def cp_wqkv(c):
        return pltpu.make_async_copy(
            wqkv_hbm.at[:, pl.ds(c * CB, CB)], wqkv.at[c], sems.at[5 + c])

    cp_mem = pltpu.make_async_copy(mem_hbm, mem0, sems.at[14])
    cp_gw = pltpu.make_async_copy(gw_hbm, gwv, sems.at[15])
    cp_woa = pltpu.make_async_copy(woa_hbm, woa, sems.at[11])

    def cp_wob(j):
        return pltpu.make_async_copy(
            wob_hbm.at[:, pl.ds(j * 128, 128)], wob.bitcast(BF16).at[j], sems.at[12])

    def start_wb(part):
        for n in range(16 * part, 16 * part + 16):
            j, i, c = n // 6, (n // 2) % 3, n % 2
            w32 = (wq_hbm, wk_hbm, wv_hbm)[i].bitcast(U32)
            pltpu.make_async_copy(
                w32.at[:, c, j, :], wb.at[j, i, c], wsems.at[j // 4]).start()

    cp_wqkv(0).start()
    cp_xa(0, SB, 0).start()

    qscale = (DA ** -0.5) * LOG2E
    nrb = S // RB

    def qk_block(c, r0, n):
        x = xa[pl.ds(r0, n), :]
        y = _dot(x, wqkv[c])
        y = (y * jnp.where(c < 2, qscale, 1.0).astype(F32)).astype(BF16)
        for g in range(CB // 128):
            qk[c * (CB // 128) + g, pl.ds(r0, n), :] = y[:, g * 128:(g + 1) * 128]

    cp_wqkv(0).wait()

    def first_body(i, carry):
        r0 = pl.multiple_of(i * SB, SB)
        cp_xa(r0, SB, i).wait()

        @pl.when(i == 0)
        def _():
            for k in range(1, RB // SB):
                cp_xa(k * SB, SB, k).start()

        @pl.when(i == 1)
        def _():
            cp_xa(RB, S - RB, 4).start()
            cp_wqkv(1).start()

        qk_block(0, r0, SB)
        return carry

    lax.fori_loop(0, RB // SB, first_body, 0)
    cp_xa(RB, S - RB, 4).wait()
    for k in range(2, 6):
        cp_wqkv(k).start()

    qk_block(0, RB, RB)

    def qk_body(i, carry):
        c = i + 1

        @pl.when(i == 0)
        def _():
            cp_wqkv(1).wait()

        @pl.when(i == 1)
        def _():
            for k in range(2, 6):
                cp_wqkv(k).wait()

        for k in range(3):
            @pl.when(i == k)
            def _():
                start_wb(2 * k)
                start_wb(2 * k + 1)

        for r in range(nrb):
            qk_block(c, r * RB, RB)
        return carry

    lax.fori_loop(0, 3, qk_body, 0)

    def v_block(i):
        c, r0 = i // nrb, (i % nrb) * RB
        quarter = wb.at[pl.ds(4 * i, 4)]
        nsub = RB // SB
        npc = NPC // nsub
        nr = (D // 2) // (NPC // 12)
        for u in range(nsub):
            y = _dot(xa[pl.ds(r0 + u * SB, SB), :], wqkv[4 + c])
            yt = y.T.astype(BF16)
            for k in range(SB // KC):
                vt[(r0 + u * SB) // KC + k, pl.ds(c * CB, CB), :] = yt[:, k * KC:(k + 1) * KC]
            for n in range(npc):
                j, rest = divmod(u * npc + n, NPC // 4)
                m, part = divmod(rest, NPC // 12)
                rows = pl.ds(part * nr, nr)
                col = (n * 4 // npc) * 128
                row = ((n * 4 % npc) // 4) * (SB * 4 // npc) // 8 * 8
                sh = ((pltpu.bitcast(y[row:row + 8, col:col + 128], U32) >> 31) >> 1) + 16
                sh = jnp.tile(sh, (nr // 8, 1))
                a = quarter[j, m, 0, rows, :]
                b = quarter[j, m, 1, rows, :]
                quarter[j, m, 0, rows, :] = (a & 0xFFFF) | (b << sh)
                quarter[j, m, 1, rows, :] = (a >> sh) | (b & jnp.uint32(0xFFFF0000))

    for j in range(8):
        cp_wob(j).start()
    cp_woa.start()
    cp_mem.start()
    cp_gw.start()
    for half in range(2):
        for i in range(2 * half, 2 * half + 2):
            quarter = wb.at[pl.ds(4 * i, 4)]
            pltpu.make_async_copy(quarter, quarter, wsems.at[i]).wait()
        for i in range(2 * half, 2 * half + 2):
            v_block(i)

    lane_grp = lax.broadcasted_iota(jnp.int32, (QB // 2, 128), 1) // DA
    qk32 = qk.bitcast(U32)
    vt32 = vt.bitcast(U32)

    def flush_tiles(g, k0, n):
        for k in range(n):
            o = ot[k0 + k, pl.ds(pl.multiple_of(g * 128, 128), 128), :]
            on[g, pl.ds(pl.multiple_of((k0 + k) * 128, 128), 128), :] = o.T.astype(BF16)

    def block_parts(na, w, nb, r, z):
        st = dict(m=None, l=None, acc=None)

        def qk_part(c):
            h = na // NQ
            if c == 0:
                qt = qk32[h // 4, pl.ds(pl.multiple_of((na % NQ) * (QB // 2), QB // 2), QB // 2), :]
                st['q'] = pltpu.bitcast(
                    jnp.where(lane_grp == h % 4, qt, jnp.zeros_like(qt)), BF16)
            kc = pltpu.bitcast(qk32[8 + h // 4, pl.ds(c * (KC // 2), KC // 2), :], BF16)
            s = _dot(kc, st['q'], NT)
            sbuf[w][pl.ds(c * KC, KC), :] = s
            for i in range(0, KC, 16):
                x = jnp.maximum(s[i:i + 8], s[i + 8:i + 16])
                st['m'] = x if st['m'] is None else jnp.maximum(st['m'], x)
            if c == NC - 1:
                mbuf[w][...] = st['m']

        def pv_part(c):
            if c == 0:
                st['mb'] = jnp.broadcast_to(
                    jnp.max(mbuf[r][...], axis=0, keepdims=True), (8, QB))
            ps = [None] * (KC // 16)
            for i in reversed(range(KC // 16)):
                base = c * KC + i * 16
                p1 = jnp.exp2(sbuf[r][pl.ds(z + base + 8, 8), :] - st['mb'])
                p0 = jnp.exp2(sbuf[r][pl.ds(z + base, 8), :] - st['mb'])
                st['l'] = p1 if st['l'] is None else st['l'] + p1
                st['l'] = st['l'] + p0
                ps[i] = jnp.concatenate([p0, p1], axis=0).astype(BF16)
            h = nb // NQ
            v = pltpu.bitcast(
                vt32[c, pl.ds(pl.multiple_of(h * (DA // 2), DA // 2), DA // 2), :], BF16)
            d = _dot(v, jnp.concatenate(ps, axis=0))
            st['acc'] = d if st['acc'] is None else st['acc'] + d
            if c == NC - 1:
                o = st['acc'] / jnp.sum(st['l'], axis=0, keepdims=True)
                for t in range(QB // 128):
                    ot[(nb % NQ) * (QB // 128) + t, pl.ds(pl.multiple_of(h * DA, DA), DA), :] = (
                        o[:, t * 128:(t + 1) * 128])

        return ([(qk_part, c) for c in range(NC)] if na is not None else [],
                [(pv_part, c) for c in range(NC)] if nb is not None else [])

    for f, c in block_parts(0, 0, None, None, None)[0]:
        f(c)
    ot[:, pl.ds(0, 128), :] = jnp.zeros((S // 128, 128, 128), F32)

    pltpu.make_async_copy(wob, wob, sems.at[12]).wait()
    cp_mem.wait()
    cp_gw.wait()

    hbuf[pl.ds(SEG, MEM), :] = mem0[...].astype(F32)
    row = lax.broadcasted_iota(jnp.int32, (LB, LB), 0)
    col = lax.broadcasted_iota(jnp.int32, (LB, LB), 1)
    mask = (row >= SEG) | (col >= SEG) | (col <= row)
    bscale = DB ** -0.5

    def step(s, last=False):
        rows = pl.ds(pl.multiple_of(s * SEG, SEG), SEG)
        hbuf[pl.ds(0, SEG), :] = xa[rows, :].astype(F32)
        z = pl.multiple_of(zero[0], 8)
        qk0, pv0 = block_parts(2 * s + 1, 1, 2 * s, 0, z)
        qk1, pv1 = block_parts(None if last else 2 * s + 2, 0, 2 * s + 1, 1, z)
        qk_parts, pv_parts = qk0 + qk1, pv0 + pv1

        def proj(h):
            w = [pltpu.bitcast(wb[h // 2, i, h % 2], BF16) for i in range(3)]
            if last:
                q = _dot(hbuf[pl.ds(0, SEG), :], w[0])
                kv = _dot(hbuf[...], jnp.concatenate(w[1:], axis=1))
            else:
                y = _dot(hbuf[...], jnp.concatenate(w, axis=1))
                q, kv = y[:, :DB], y[:, DB:]
            return _round(q), kv[:, :DB].astype(BF16), kv[:, DB:].astype(BF16)

        def scores(q, k):
            sc = jnp.where(mask[:q.shape[0]], _dot(q, k, NT) * bscale, -1000000000.0)
            e = jnp.exp(sc - jnp.max(sc, axis=1, keepdims=True))
            return _round(e), jnp.sum(e, axis=1, keepdims=True)

        def attend(e, l, v):
            return _round(_dot(e, v) / l)

        def oproj(h, o):
            w = jnp.concatenate(
                [pltpu.bitcast(wob[j, pl.ds(h * (DB // 2), DB // 2), :], BF16)
                 for j in range(D // 128)], axis=1)
            return _dot(o, w)

        qkv, el, oo = {}, {}, {}
        acc = None
        for t in range(HB + 5):
            if t == 30:
                flush_tiles(jnp.maximum(s // 8 - 1, 0), (s % 8) * 2, 2)
                gw = gwv[...].reshape(1, D).astype(F32)
                g = jax.nn.sigmoid(
                    jnp.sum(hbuf[pl.ds(0, SEG), :] * gw, axis=1, keepdims=True))
                gate[rows, :] = jnp.broadcast_to(g, (SEG, 128))
            if t in ATT_SLOTS:
                for parts in (qk_parts, pv_parts):
                    for f, c in parts[ATT_SLOTS.index(t):][:1]:
                        f(c)
            if t < HB:
                qkv[t] = proj(t)
            if 0 <= t - 1 < HB:
                el[t - 1] = scores(qkv[t - 1][0], qkv[t - 1][1])
            if 0 <= t - 3 < HB:
                oo[t - 3] = attend(*el[t - 3], qkv[t - 3][2])
            if 0 <= t - 5 < HB:
                y = oproj(t - 5, oo[t - 5])
                acc = y if acc is None else acc + y
        if not last:
            hbuf[pl.ds(SEG, MEM), :] = _round(acc[SEG:])
        bout[rows, :] = (1.0 - g) * acc[:SEG]

    def step_body(s, carry):
        step(s)
        return carry

    zero[0] = 0
    lax.fori_loop(0, NSEG - 1, step_body, 0)
    step(NSEG - 1, last=True)
    flush_tiles(HA // 4 - 1, 0, S // 128)

    cp_woa.wait()

    r0 = 0
    for n in (512, 512, 512, 256, 128, 64, 64):
        rows = pl.ds(r0, n)
        o = jnp.concatenate([on[k, rows, :] for k in range(D // 128)], axis=1)
        a = _dot(o, woa[...])
        g = jnp.tile(gate[rows, :], (1, D // 128))
        outv[rows, :] = (g * a + bout[rows, :]).astype(BF16)
        pltpu.make_async_copy(outv.at[rows], out_hbm.at[rows], sems.at[13]).start()
        r0 += n
    assert r0 == S
    pltpu.make_async_copy(outv, out_hbm, sems.at[13]).wait()


@jax.jit
def pallas_gated_mix__softmax_full_mha__memory_aug_recurrent_mem_tr__prompt_kernel(
    A_x, A_wqkv, A_wo, B_x, B_mem0, B_Wq, B_Wk, B_Wv, B_Wo, B_seg_len, gate_w,
):
    del B_x
    del B_seg_len
    hbm = pl.BlockSpec(memory_space=pl.ANY)
    split_d = (D // 2, 2, HB, DB)
    out = pl.pallas_call(
        _kernel,
        out_shape=jax.ShapeDtypeStruct((S, D), BF16),
        in_specs=[hbm] * 9,
        out_specs=hbm,
        scratch_shapes=[
            pltpu.VMEM((S, D), BF16),
            pltpu.VMEM((3 * D // CB, D, CB), BF16),
            pltpu.VMEM((D, D), BF16),
            pltpu.VMEM((HB // 2, 3, 2, D // 2, 128), U32),
            pltpu.VMEM((D // 128, HB * DB // 2, 128), U32),
            pltpu.VMEM((16, S, 128), BF16),
            pltpu.VMEM((NC, D, KC), BF16),
            pltpu.VMEM((S // 128, D, 128), F32),
            pltpu.VMEM((D // 128, S, 128), BF16),
            [pltpu.VMEM((S, QB), F32) for _ in range(2)],
            [pltpu.VMEM((8, QB), F32) for _ in range(2)],
            pltpu.VMEM((S, D), F32),
            pltpu.VMEM((S, 128), F32),
            pltpu.VMEM((LB, D), F32),
            pltpu.VMEM((S, D), BF16),
            pltpu.VMEM((MEM, D), BF16),
            pltpu.VMEM((D,), BF16),
            pltpu.SMEM((1,), jnp.int32),
            pltpu.SemaphoreType.DMA((16,)),
            pltpu.SemaphoreType.DMA((4,)),
        ],
        compiler_params=pltpu.CompilerParams(vmem_limit_bytes=120 * 1024 * 1024),
        name="gated_mix",
    )(
        A_x.reshape(S, D), A_wqkv, A_wo, B_mem0.reshape(MEM, D),
        B_Wq.reshape(split_d), B_Wk.reshape(split_d), B_Wv.reshape(split_d),
        B_Wo.reshape(HB * DB, D), gate_w,
    )
    return out.reshape(1, S, D)
```
